```python
import os as _os
_os.environ.setdefault("JAX_PLATFORMS", "cpu")
import jax
import jax.numpy as jnp

def _softmax(x, axis=-1):
    return jax.nn.softmax(x, axis=axis)
def _gelu(x):
    return jax.nn.gelu(x, approximate=True)
def _silu(x):
    return jax.nn.silu(x)
def _sigmoid(x):
    return jax.nn.sigmoid(x)
def _layernorm(x, axis=-1, eps=1e-5):
    m = jnp.mean(x, axis=axis, keepdims=True)
    v = jnp.var(x, axis=axis, keepdims=True)
    return (x - m) / jnp.sqrt(v + eps)
def _scatter_add(tgt, idx, src, axis=0):
    return tgt.at[idx].add(src)
def _segment_sum(src, seg, n):
    return jax.ops.segment_sum(src, seg, n)
class _Rng:
    def __init__(self, key):
        self._k = key
    def _next(self):
        self._k, sub = jax.random.split(self._k)
        return sub
    def normal(self, shape):
        return jax.random.normal(self._next(), shape, dtype=jnp.bfloat16)
    def randint(self, lo, hi, shape):
        return jax.random.randint(self._next(), shape, lo, hi, dtype=jnp.int32)
    def uniform(self, shape, lo=0.0, hi=1.0):
        return jax.random.uniform(self._next(), shape, jnp.bfloat16, lo, hi)
    def permutation(self, n):
        return jax.random.permutation(self._next(), n)


kernel_name = 'gated_mix__softmax_full_mha__spectral_gfnet__prompt'

def setup_inputs():
    _rng = _Rng(jax.random.key(int.from_bytes(__import__("os").urandom(4), "little")))
    _w = (lambda a: (lambda t: t.astype(jnp.bfloat16) if jnp.issubdtype(t.dtype, jnp.floating) else t)(jnp.asarray(a)))
    def _A_setup():
        B, S, D = 1, 2048, 448
        return {
            "x": _w((lambda *s: _rng.normal(s) * 0.05)(B, S, D)),
            "wqkv": _w((lambda *s: _rng.normal(s) * 0.4)(D, 3 * D)),
            "wo": _w((lambda *s: _rng.normal(s) * 0.05)(D, D)),
        }
    _A_in = _A_setup()

    def _B_setup():
        B, S, D = 1, 2048, 448
        Df = D // 2 + 1
        return {
            "x": _w((lambda *s: _rng.normal(s) * 0.05)(B, S, D)),
            "w_r": _w((lambda *s: _rng.normal(s) * 1.6)(S, Df) * 0.02),
            "w_i": _w((lambda *s: _rng.normal(s) * 1.6)(S, Df) * 0.02),
        }
    _B_in = _B_setup()

    return {
        "A_x": _A_in["x"],
        "A_wqkv": _A_in["wqkv"],
        "A_wo": _A_in["wo"],
        "B_x": _B_in["x"],
        "B_w_r": _B_in["w_r"],
        "B_w_i": _B_in["w_i"],
        "gate_w": _w((lambda *s: _rng.normal(s) * 0.05)(448) * 16.0),
    }

def reference(A_x, A_wqkv, A_wo, B_x, B_w_r, B_w_i, gate_w):
    def _A_ref(x, wqkv, wo):
        B, S, D = x.shape
        H = 16; Dh = D // H
        qkv = (lambda x, *d: x.transpose(*d))((x @ wqkv).reshape(B, S, 3, H, Dh), 2, 0, 3, 1, 4)
        q, k, v = qkv[0], qkv[1], qkv[2]
        scale = Dh ** -0.5
        scores = jnp.einsum("bhqd,bhkd->bhqk", q, k) * scale
        p = _softmax(scores, axis=-1)
        o = jnp.einsum("bhqk,bhkd->bhqd", p, v)
        return (lambda x, *d: x.transpose(*d))(o, 0, 2, 1, 3).reshape(B, S, D) @ wo

    def _B_ref(x, w_r, w_i):
        B, S, D = x.shape
        X = (lambda x, axes=(-2,-1): jnp.fft.rfft2(x.astype(jnp.float32), axes=axes))(x, axes=(-2, -1))
        W = w_r + 1j * w_i
        X = X * W
        y = (lambda x, s, axes=(-2,-1): jnp.fft.irfft2(x, s=s, axes=axes).astype(jnp.bfloat16))(X, (S, D), axes=(-2, -1))
        return y

    x = A_x
    g = _sigmoid((x * gate_w).sum(-1, keepdims=True))
    a = _A_ref(x, A_wqkv, A_wo)
    b = _B_ref(x, B_w_r, B_w_i)
    return g * a + (1 - g) * b
```

```python
import math
import numpy as np
import jax
import jax.numpy as jnp
from jax.experimental import pallas as pl
from jax.experimental.pallas import tpu as pltpu

S, D, H, DH = 2048, 448, 16, 28
DF = D // 2 + 1
LP = 240
N1, N2 = 16, 128
QSCALE = DH ** -0.5 * math.log2(math.e)
F32, BF16, I32 = jnp.float32, jnp.bfloat16, jnp.int32
L_LO, L_HI = 2.0 ** -64, 2.0 ** 64
DEBUG = ""


def _constants():
    l = np.arange(DF)[:, None]
    d = np.arange(D)[None, :]
    ang = 2 * np.pi * ((l * d) % D) / D
    FT = np.zeros((2 * LP, D))
    FT[:DF] = np.cos(ang)
    FT[LP:LP + DF] = -np.sin(ang)
    c = np.full((DF, 1), 2.0); c[0] = 1.0; c[-1] = 1.0
    Gt = np.zeros((D, 2 * LP))
    Gt[:, :DF] = (c * np.cos(ang)).T / (D * S)
    sn = -c * np.sin(ang); sn[0] = 0.0; sn[-1] = 0.0
    Gt[:, LP:LP + DF] = sn.T / (D * S)
    n2 = np.arange(N2)[:, None]; k2 = np.arange(N2)[None, :]
    Mf = np.zeros((N1, 2 * N2, 2 * N2))
    for k1 in range(N1):
        th = 2 * np.pi * ((n2 * k2 * N1 + n2 * k1) % S) / S
        Tr, Ti = np.cos(th), -np.sin(th)
        Mf[k1] = np.block([[Tr, Ti], [-Ti, Tr]])
    return jnp.asarray(FT, BF16), jnp.asarray(Gt, BF16), jnp.asarray(Mf, BF16)


def _cmul_const(re, im, k, n, sign):
    k = k % n
    if k == 0:
        return re, im
    if 4 * k == n:
        return (-im, re) if sign > 0 else (im, -re)
    if 2 * k == n:
        return -re, -im
    if 4 * k == 3 * n:
        return (im, -re) if sign > 0 else (-im, re)
    c = math.cos(2 * math.pi * k / n); s = sign * math.sin(2 * math.pi * k / n)
    if (8 * k) % n == 0:
        a = abs(c)
        sc, ss = (1 if c > 0 else -1), (1 if s > 0 else -1)
        rr = (re - im) if sc == ss else (re + im)
        ii = (re + im) if sc == ss else (im - re)
        return rr * (sc * a), ii * (sc * a)
    return re * c - im * s, re * s + im * c


def _fft(xs, sign):
    n = len(xs)
    if n == 1:
        return xs
    ev = _fft(xs[0::2], sign)
    od = _fft(xs[1::2], sign)
    out = [None] * n
    for k in range(n // 2):
        tr, ti = _cmul_const(od[k][0], od[k][1], k, n, sign)
        out[k] = (ev[k][0] + tr, ev[k][1] + ti)
        out[k + n // 2] = (ev[k][0] - tr, ev[k][1] - ti)
    return out


def _nt(a, b):
    return jax.lax.dot_general(a, b, (((1,), (1,)), ((), ())), preferred_element_type=F32)


def _nn(a, b):
    return jnp.dot(a, b, preferred_element_type=F32)


KC = 128
SKEW = 2


def _kernel(xa_ref, wqkv_ref, wo_ref, wr_ref, wi_ref, gw_ref, ft_ref, gt_ref, mf_ref,
            out_ref,
            k_scr, qt_scr, vt_scr, negm_scr, g_scr, l_scr, ot_scr, wot_scr,
            u_scr, a_scr, b_scr, z_scr, wn_scr, wp_scr):
    wT = wqkv_ref[...].astype(F32).T
    z4 = jnp.zeros((4, D), F32)
    z1 = jnp.zeros((1, D), F32)
    parts = []
    for h in range(H):
        parts.append(wT[2 * D + DH * h: 2 * D + DH * h + DH, :])
        if h == 0:
            parts += [z1, gw_ref[...].astype(F32), z1, z1]
        else:
            parts.append(z4)
    wvT_pad = jnp.concatenate(parts, axis=0).astype(BF16)
    wqkT = wT[0:2 * D + 16, :].astype(BF16)
    wo = wo_ref[...].astype(F32)
    parts = []
    for h in range(H):
        parts += [wo[DH * h: DH * h + DH, :], z4]
    wo_pad = jnp.concatenate(parts, axis=0)
    wot_scr[...] = jnp.concatenate([wo_pad, jnp.zeros((512, 64), F32)], axis=1).T[:D, :].astype(BF16)

    xa = xa_ref[...]
    qk = _nn(wqkT, xa)
    qt = (qk[0:D + 16] * QSCALE).astype(BF16)
    qt_scr[...] = qt
    lane = jax.lax.broadcasted_iota(I32, (S, 128), 1)
    hh = jax.lax.broadcasted_iota(I32, (8, 128), 0)
    ll = jax.lax.broadcasted_iota(I32, (8, 128), 1)
    for g in range(4):
        kg = qk[D + 112 * g: D + 112 * g + 128, :].T
        kg = jnp.where(lane == 112, 1.0, kg).astype(BF16)
        k_scr[:, 128 * g:128 * g + 128] = kg
        kmax = jnp.max(jnp.abs(kg.astype(F32)), axis=0, keepdims=True)
        ind = jnp.where((ll >= hh * DH) & (ll < hh * DH + DH) & (hh < 4), kmax * 1.02, 0.0).astype(BF16)
        mt = _nn(ind, jnp.abs(qt[112 * g:112 * g + 128, :]))
        negm_scr[4 * g:4 * g + 4, :] = -mt[0:4]
    vt = _nn(wvT_pad, xa)
    g_scr[...] = jax.nn.sigmoid(vt[29:30, :])
    row = jax.lax.broadcasted_iota(I32, (512, S), 0)
    vt = jnp.where(row % 32 == 28, 1.0, vt)
    vt = jnp.where(row == 29, 0.0, vt)
    vt_scr[...] = vt.astype(BF16)

    def masked_q(h, q0, tq, with_shift):
        g = h // 4
        r0 = pl.multiple_of(g * 112, 16)
        g0 = pl.multiple_of(g * 128, 128)
        j0 = (h % 4) * DH
        qs = qt_scr[pl.ds(r0, 128), pl.ds(q0, tq)]
        rows = jax.lax.broadcasted_iota(I32, (128, tq), 0)
        qm = jnp.where((rows >= j0) & (rows < j0 + DH), qs.astype(F32), 0.0)
        if with_shift:
            qm = jnp.where(rows == 112, negm_scr[pl.ds(h, 1), pl.ds(q0, tq)], qm)
        return qm.astype(BF16), g0

    def head_body(h, carry):
        h0 = pl.multiple_of(h * 32, 32)
        qm, g0 = masked_q(h, 0, S, True)
        nc = S // KC
        ps = {}
        acc = None
        for i in range(nc + SKEW):
            if i < nc:
                s = _nn(k_scr[pl.ds(i * KC, KC), pl.ds(g0, 128)], qm)
                ps[i] = jnp.exp2(s).astype(BF16)
            if i >= SKEW:
                c = i - SKEW
                ov = _nn(vt_scr[pl.ds(h0, 32), pl.ds(c * KC, KC)], ps.pop(c))
                acc = ov if acc is None else acc + ov
        l = acc[28:29, :]
        l_scr[pl.ds(h, 1), :] = l
        ot_scr[pl.ds(h0, 32), :] = (acc * (g_scr[...] / l)).astype(BF16)
        return carry

    jax.lax.fori_loop(0, H, head_body, 0)

    lv = l_scr[...]
    bad = jnp.where((lv >= L_LO) & (lv <= L_HI), 0.0, 1.0)
    nbad = jnp.max(bad)

    @pl.when(nbad > 0.5)
    def _():
        TQ = 128
        def item(it, carry):
            h = it // (S // TQ)
            q0 = pl.multiple_of((it % (S // TQ)) * TQ, TQ)
            h0 = pl.multiple_of(h * 32, 32)
            qm, g0 = masked_q(h, q0, TQ, False)
            s = _nn(k_scr[:, pl.ds(g0, 128)], qm)
            m = jnp.max(s, axis=0, keepdims=True)
            p = jnp.exp2(s - m).astype(BF16)
            acc = _nn(vt_scr[pl.ds(h0, 32), :], p)
            l = acc[28:29, :]
            ot_scr[pl.ds(h0, 32), pl.ds(q0, TQ)] = (acc * (g_scr[:, pl.ds(q0, TQ)] / l)).astype(BF16)
            return carry
        jax.lax.fori_loop(0, H * (S // TQ), item, 0)

    u_scr[...] = _nn(ft_ref[...], xa_ref[...])
    wrb = pltpu.bitcast(wr_ref[...].astype(F32), I32)
    wib = pltpu.bitcast(wi_ref[...].astype(F32), I32)
    wpk = wrb | jax.lax.shift_right_logical(wib, 16)
    wpk = jnp.concatenate([wpk, jnp.zeros((256 - DF, S), I32)], axis=0)
    wn = wpk.T
    wn_scr[0] = wn[:, 0:128]
    wn_scr[1] = wn[:, 128:256]
    for k1 in range(N1):
        for t in range(2):
            wp_scr[k1, 128 * t:128 * t + 128, :] = wn_scr[t, pl.ds(k1, N2, stride=N1), :].T

    xs = [(u_scr[0:LP, 128 * n:128 * n + 128], u_scr[LP:2 * LP, 128 * n:128 * n + 128]) for n in range(N1)]
    ys = _fft(xs, -1)
    for k1 in range(N1):
        a_scr[k1, :, 0:128] = ys[k1][0].astype(BF16)
        a_scr[k1, :, 128:256] = ys[k1][1].astype(BF16)

    for k1 in range(N1):
        x = _nn(a_scr[k1], mf_ref[k1])
        xr, xi = x[:, :128], x[:, 128:]
        w = wp_scr[k1, 0:LP, :]
        wr = pltpu.bitcast(w & jnp.int32(-65536), F32)
        wi = pltpu.bitcast(jax.lax.shift_left(w, 16), F32)
        y = jnp.concatenate([xr * wr - xi * wi, xr * wi + xi * wr], axis=1).astype(BF16)
        b_scr[k1] = _nt(y, mf_ref[k1])

    xs = [(b_scr[k1, :, 0:128], b_scr[k1, :, 128:256]) for k1 in range(N1)]
    ys = _fft(xs, +1)
    for n in range(N1):
        z_scr[0:LP, 128 * n:128 * n + 128] = ys[n][0].astype(BF16)
        z_scr[LP:2 * LP, 128 * n:128 * n + 128] = ys[n][1].astype(BF16)

    at = _nn(wot_scr[...], ot_scr[...])
    bt = _nn(gt_ref[...], z_scr[...])
    if DEBUG == "a":
        out_ref[...] = at.astype(BF16)
    elif DEBUG == "b":
        out_ref[...] = bt.astype(BF16)
    else:
        out_ref[...] = (at + (1.0 - g_scr[...]) * bt).astype(BF16)


@jax.jit
def pallas_gated_mix__softmax_full_mha__spectral_gfnet__prompt_kernel(A_x, A_wqkv, A_wo, B_x, B_w_r, B_w_i, gate_w):
    FT, Gt, Mf = _constants()
    out = pl.pallas_call(
        _kernel,
        out_shape=jax.ShapeDtypeStruct((D, S), BF16),
        scratch_shapes=[
            pltpu.VMEM((S, 512), BF16),
            pltpu.VMEM((D + 16, S), BF16),
            pltpu.VMEM((512, S), BF16),
            pltpu.VMEM((H, S), F32),
            pltpu.VMEM((1, S), F32),
            pltpu.VMEM((H, S), F32),
            pltpu.VMEM((512, S), BF16),
            pltpu.VMEM((D, 512), BF16),
            pltpu.VMEM((2 * LP, S), F32),
            pltpu.VMEM((N1, LP, 256), BF16),
            pltpu.VMEM((N1, LP, 256), F32),
            pltpu.VMEM((2 * LP, S), BF16),
            pltpu.VMEM((2, S, 128), I32),
            pltpu.VMEM((N1, 256, 128), I32),
        ],
        compiler_params=pltpu.CompilerParams(vmem_limit_bytes=110 * 1024 * 1024),
    )(A_x.reshape(S, D).T, A_wqkv, A_wo, B_w_r.T, B_w_i.T, gate_w.reshape(1, D), FT, Gt, Mf)
    return out.T.reshape(1, S, D)
```

```python
import math
import numpy as np
import jax
import jax.numpy as jnp
from jax.experimental import pallas as pl
from jax.experimental.pallas import tpu as pltpu

S, D, H, DH = 2048, 448, 16, 28
DF = D // 2 + 1
LP = 256
N1, N2 = 16, 128
QSCALE = DH ** -0.5 * math.log2(math.e)
F32, BF16, I32 = jnp.float32, jnp.bfloat16, jnp.int32
L_LO, L_HI = 2.0 ** -64, 2.0 ** 64
CLS = ((0, 0, 64, 57), (2, 64, 56, 56), (1, 120, 56, 56), (3, 176, 56, 56))
NREAL = 232


def _constants():
    d0 = np.arange(112)[None, :]

    def cs(cls, n_real, n_pad):
        l = (cls + 4 * np.arange(n_real))[:, None]
        th = 2 * np.pi * ((l * d0) % D) / D
        c = np.zeros((n_pad, 112)); s = np.zeros((n_pad, 112))
        c[:n_real] = np.cos(th); s[:n_real] = np.sin(th)
        w = np.zeros((n_pad, 1)); w[:n_real] = 2.0
        w[:n_real][(l == 0) | (l == D // 2)] = 1.0
        return c, s, w
    c0, s0, w0 = cs(0, 57, 64); c2, s2, w2 = cs(2, 56, 56); c1, s1, w1 = cs(1, 56, 56); c3, s3, w3 = cs(3, 56, 56)
    F02 = np.concatenate([c0, -s0, c2, -s2], axis=0)
    F13 = np.block([[c1, -s1], [-s1, -c1], [c3, s3], [-s3, c3]])
    nrm = 1.0 / (D * S)
    G0 = np.concatenate([(w0 * c0).T, (-w0 * s0).T], axis=1) * nrm
    G2 = np.concatenate([(w2 * c2).T, (-w2 * s2).T], axis=1) * nrm
    G13 = np.block([[(w1 * c1).T, (-w1 * s1).T, (w3 * c3).T, (-w3 * s3).T],
                    [(-w1 * s1).T, (-w1 * c1).T, (w3 * s3).T, (w3 * c3).T]]) * nrm
    G02 = np.zeros((224, 128)); G02[:112] = G0; G02[112:, :112] = G2
    n2 = np.arange(N2)[:, None]; k2 = np.arange(N2)[None, :]
    th = 2 * np.pi * ((n2 * k2) % N2) / N2
    Fr, Fi = np.cos(th), -np.sin(th)
    FF = np.where(n2 <= N2 // 2, np.cos(th), np.sin(th))
    FF[0] *= 0.5; FF[N2 // 2] *= 0.5
    k1 = np.arange(N1)[:, None]
    tt = 2 * np.pi * ((k1 * np.arange(N2)[None, :]) % S) / S
    TW = np.concatenate([np.cos(tt), -np.sin(tt)], axis=0)
    return tuple(jnp.asarray(m, BF16) for m in (F02, F13, G02, G13, FF)) + (jnp.asarray(TW, F32),)


def _cmul_const(re, im, k, n, sign):
    k = k % n
    if k == 0:
        return re, im
    if 4 * k == n:
        return (-im, re) if sign > 0 else (im, -re)
    if 2 * k == n:
        return -re, -im
    if 4 * k == 3 * n:
        return (im, -re) if sign > 0 else (-im, re)
    c = math.cos(2 * math.pi * k / n); s = sign * math.sin(2 * math.pi * k / n)
    if (8 * k) % n == 0:
        a = abs(c)
        sc, ss = (1 if c > 0 else -1), (1 if s > 0 else -1)
        rr = (re - im) if sc == ss else (re + im)
        ii = (re + im) if sc == ss else (im - re)
        return rr * (sc * a), ii * (sc * a)
    return re * c - im * s, re * s + im * c


def _fft(xs, sign):
    n = len(xs)
    if n == 1:
        return xs
    ev = _fft(xs[0::2], sign)
    od = _fft(xs[1::2], sign)
    out = [None] * n
    for k in range(n // 2):
        tr, ti = _cmul_const(od[k][0], od[k][1], k, n, sign)
        out[k] = (ev[k][0] + tr, ev[k][1] + ti)
        out[k + n // 2] = (ev[k][0] - tr, ev[k][1] - ti)
    return out


def _nt(a, b):
    return jax.lax.dot_general(a, b, (((1,), (1,)), ((), ())), preferred_element_type=F32)


def _nn(a, b):
    return jnp.dot(a, b, preferred_element_type=F32)


def _rev(x):
    lane = jax.lax.broadcasted_iota(I32, x.shape, 1)
    return jnp.take_along_axis(x, (N2 - lane) % N2, axis=1)


def _fold(re, im, sign):
    lane = jax.lax.broadcasted_iota(I32, re.shape, 1)
    lo = lane <= N2 // 2
    rr, ri = _rev(re), _rev(im)
    if sign < 0:
        return jnp.where(lo, re + rr, im - ri), jnp.where(lo, im + ri, rr - re)
    return jnp.where(lo, re + rr, ri - im), jnp.where(lo, im + ri, re - rr)


KC = 128
SKEW = 2
HP = 2
RG = LP // (H // HP)
KP = 1
NP = N1 // KP
NSPL = 2
ISTEP = 2
ST_X = 2
ST_Y = 6
ST_I = 26
XCH = 4
XW = S // XCH
OCH = 8
OW = S // OCH


def _kernel(xa_hbm, wqkv_hbm, wo_hbm, wr_hbm, wi_hbm, gw_ref, f02_hbm, f13_hbm, g02_hbm, g13_hbm, mf_hbm, tw_ref,
            out_hbm,
            x_v, wqk_v, wv_v, wo_v, wr_v, wi_v, f02_v, f13_v, g02_v, g13_v, mf_v, out_v, sems,
            k_scr, qt_scr, vt_scr, negm_scr, g_scr, l_scr, ot_scr, wot_scr,
            u_scr, z_scr, wn_scr, wp_scr, wc_scr, fa_scr, fx_scr, fb_scr, p_scr):
    nsem = [0]

    def cp(src, dst):
        nsem[0] += 1
        return pltpu.make_async_copy(src, dst, sems.at[nsem[0] - 1])

    c_wqk = cp(wqkv_hbm.at[:, pl.ds(0, 1024)], wqk_v)
    c_f = [cp(f02_hbm, f02_v), cp(f13_hbm, f13_v)]
    c_x = [cp(xa_hbm.at[:, pl.ds(c * XW, XW)], x_v.at[:, pl.ds(c * XW, XW)]) for c in range(XCH)]
    rest = [cp(wqkv_hbm.at[:, pl.ds(896, 448)], wv_v), cp(wr_hbm, wr_v), cp(wi_hbm, wi_v), cp(mf_hbm, mf_v),
            cp(wo_hbm, wo_v), cp(g02_hbm, g02_v), cp(g13_hbm, g13_v)]
    c_out = [cp(out_v.at[:, pl.ds(c * OW, OW)], out_hbm.at[:, pl.ds(c * OW, OW)]) for c in range(OCH)]
    c_wqk.start()
    for c in c_f:
        c.start()
    c_x[0].start()
    c_wqk.wait()
    for c in c_x[1:]:
        c.start()

    wqkT = wqk_v[...].astype(F32).T[0:2 * D + 16, :].astype(BF16)

    lane = jax.lax.broadcasted_iota(I32, (XW, 128), 1)
    kmax = [None] * 4

    def dfwd(c):
        cols = slice(c * XW, (c + 1) * XW)
        xf = x_v[:, cols].astype(F32)
        x0, x1, x2, x3 = (xf[112 * j:112 * j + 112] for j in range(4))
        s02, s13 = x0 + x2, x1 + x3
        e0 = (s02 + s13).astype(BF16)
        e2 = (s02 - s13).astype(BF16)
        ab = jnp.concatenate([x0 - x2, x1 - x3], axis=0).astype(BF16)
        r0 = _nn(f02_v[0:128, :], e0)
        r2 = _nn(f02_v[128:240, :], e2)
        r13 = _nn(f13_v[...], ab)
        zpad = jnp.zeros((LP - NREAL, XW), F32)
        u_scr[0:LP, cols] = jnp.concatenate([r0[0:64], r2[0:56], r13[0:56], r13[112:168], zpad], axis=0)
        u_scr[LP:2 * LP, cols] = jnp.concatenate([r0[64:128], r2[56:112], r13[56:112], r13[168:224], zpad], axis=0)

    def qkproj(c):
        cols = slice(c * XW, (c + 1) * XW)
        qk = _nn(wqkT, x_v[:, cols])
        qt_scr[:, cols] = (qk[0:D + 16] * QSCALE).astype(BF16)
        for g in range(4):
            kg = qk[D + 112 * g: D + 112 * g + 128, :].T
            kg = jnp.where(lane == 112, 1.0, kg)
            k_scr[cols, 128 * g:128 * g + 128] = kg.astype(BF16)
            km = jnp.max(jnp.abs(kg), axis=0, keepdims=True)
            kmax[g] = km if kmax[g] is None else jnp.maximum(kmax[g], km)

    def wshuf_first():
        wrb = pltpu.bitcast(wr_v[...].astype(F32), I32)
        wib = pltpu.bitcast(wi_v[...].astype(F32), I32)
        wpk = wrb | jax.lax.shift_right_logical(wib, 16)
        wpk = jnp.concatenate([wpk, jnp.zeros((256 - DF, S), I32)], axis=0)
        wn = wpk.T
        wn_scr[0] = wn[:, 0:128]
        wn_scr[1] = wn[:, 128:256]

    def wshuf_second(k1):
        for t in range(2):
            wp_scr[k1, 128 * t:128 * t + 128, :] = wn_scr[t, pl.ds(k1, N2, stride=N1), :].T
        wc_scr[k1] = jnp.concatenate([wp_scr[k1, pl.ds(c, n, stride=4), :] for c, _, n, _ in CLS]
                                     + [jnp.zeros((LP - NREAL, 128), I32)], axis=0)

    for c in range(XCH - 1):
        if c == 0:
            for cf in c_f:
                cf.wait()
        c_x[c].wait()
        if c == 0:
            for cr in rest:
                cr.start()
        qkproj(c)
        dfwd(c)

    c_x[XCH - 1].wait()
    for cr in rest:
        cr.wait()

    qkproj(XCH - 1)
    dfwd(XCH - 1)
    wvT = wv_v[...].astype(F32).T
    z4 = jnp.zeros((4, D), F32)
    z1 = jnp.zeros((1, D), F32)
    parts = []
    for h in range(H):
        parts.append(wvT[DH * h: DH * h + DH, :])
        if h == 0:
            parts += [z1, gw_ref[...].astype(F32).reshape(1, D), z1, z1]
        else:
            parts.append(z4)
    wvT_pad = jnp.concatenate(parts, axis=0).astype(BF16)
    wshuf_first()

    row = jax.lax.broadcasted_iota(I32, (512, XW), 0)
    for c in range(XCH):
        cols = slice(c * XW, (c + 1) * XW)
        vt = _nn(wvT_pad, x_v[:, cols])
        g_scr[:, cols] = jax.nn.sigmoid(vt[29:30, :])
        vt = jnp.where(row % 32 == 28, 1.0, vt)
        vt = jnp.where(row == 29, 0.0, vt)
        vt_scr[:, cols] = vt.astype(BF16)
        for k1 in range(4 * c, 4 * c + 4):
            wshuf_second(k1)

    hh = jax.lax.broadcasted_iota(I32, (8, 128), 0)
    ll = jax.lax.broadcasted_iota(I32, (8, 128), 1)
    for g in range(4):
        ind = jnp.where((ll >= hh * DH) & (ll < hh * DH + DH) & (hh < 4), kmax[g] * 1.02, 0.0).astype(BF16)
        mt = _nn(ind, jnp.abs(qt_scr[112 * g:112 * g + 128, :]))
        negm_scr[4 * g:4 * g + 4, :] = -mt[0:4]

    wo = wo_v[...].astype(F32)
    parts = []
    for h in range(H):
        parts += [wo[DH * h: DH * h + DH, :], z4]
    wo_pad = jnp.concatenate(parts, axis=0)
    wot_scr[...] = jnp.concatenate([wo_pad, jnp.zeros((512, 64), F32)], axis=1).T[:D, :].astype(BF16)

    def masked_q(h, q0, tq, with_shift):
        g = h // 4
        r0 = pl.multiple_of(g * 112, 16)
        g0 = pl.multiple_of(g * 128, 128)
        j0 = (h % 4) * DH
        qs = qt_scr[pl.ds(r0, 128), pl.ds(q0, tq)]
        rows = jax.lax.broadcasted_iota(I32, (128, tq), 0)
        qm = jnp.where((rows >= j0) & (rows < j0 + DH), qs.astype(F32), 0.0)
        if with_shift:
            qm = jnp.where(rows == 112, negm_scr[pl.ds(h, 1), pl.ds(q0, tq)], qm)
        return qm.astype(BF16), g0

    def head_body(t, carry):
        nc = S // KC
        seq = [(u, c) for u in range(HP) for c in range(nc)]
        qms = {}
        accs = {}
        r0 = pl.multiple_of(t * RG, 16)
        for i in range(len(seq) + SKEW):
            if i < NSPL:
                sr = RG // NSPL
                ro = i * sr
                xs = [(u_scr[pl.ds(r0 + ro, sr), 128 * n:128 * n + 128],
                       u_scr[pl.ds(LP + r0 + ro, sr), 128 * n:128 * n + 128]) for n in range(N1)]
                ys = _fft(xs, -1)
                for k1 in range(N1):
                    ar, ai = ys[k1]
                    if k1 > 0:
                        tr, ti = tw_ref[k1:k1 + 1, :], tw_ref[N1 + k1:N1 + k1 + 1, :]
                        ar, ai = ar * tr - ai * ti, ar * ti + ai * tr
                    f1, f2 = _fold(ar, ai, -1)
                    fa_scr[2 * RG * k1 + ro:2 * RG * k1 + ro + sr, :] = f1.astype(BF16)
                    fa_scr[2 * RG * k1 + RG + ro:2 * RG * k1 + RG + ro + sr, :] = f2.astype(BF16)
            if i < len(seq):
                u, c = seq[i]
                h = HP * t + u
                if c == 0:
                    qms[u] = masked_q(h, 0, S, True)
                qm, g0 = qms[u]
                s = _nn(k_scr[pl.ds(c * KC, KC), pl.ds(g0, 128)], qm)
                p_scr[i % (SKEW + 1)] = jnp.exp2(s).astype(BF16)
            if i >= SKEW:
                u, c = seq[i - SKEW]
                h = HP * t + u
                h0 = pl.multiple_of(h * 32, 32)
                ov = _nn(vt_scr[pl.ds(h0, 32), pl.ds(c * KC, KC)], p_scr[(i - SKEW) % (SKEW + 1)])
                accs[u] = ov if u not in accs else accs[u] + ov
                if c == nc - 1:
                    acc = accs[u]
                    l = acc[28:29, :]
                    l_scr[pl.ds(h, 1), :] = l
                    ot_scr[pl.ds(h0, 32), :] = (acc * (g_scr[...] / l)).astype(BF16)
            if True:
                p = i - ST_X
                if 0 <= p < NP:
                    rows_ = slice(2 * RG * KP * p, 2 * RG * KP * (p + 1))
                    fx_scr[rows_, :] = _nn(fa_scr[rows_, :], mf_v[...])
                p = i - ST_Y
                if 0 <= p < NP:
                    x = fx_scr[2 * RG * KP * p:2 * RG * KP * (p + 1), :]
                    ys_ = []
                    for j, k1 in enumerate(range(p * KP, (p + 1) * KP)):
                        xr, xi = x[2 * j * RG:(2 * j + 1) * RG], x[(2 * j + 1) * RG:(2 * j + 2) * RG]
                        w = wc_scr[k1, pl.ds(r0, RG), :]
                        wr = pltpu.bitcast(w & jnp.int32(-65536), F32)
                        wi = pltpu.bitcast(jax.lax.shift_left(w, 16), F32)
                        f1, f2 = _fold(xr * wr - xi * wi, xr * wi + xi * wr, +1)
                        ys_ += [f1, f2]
                    b = _nn(jnp.concatenate(ys_, axis=0).astype(BF16), mf_v[...])
                    for j, k1 in enumerate(range(p * KP, (p + 1) * KP)):
                        br, bi = b[2 * j * RG:(2 * j + 1) * RG], b[(2 * j + 1) * RG:(2 * j + 2) * RG]
                        if k1 > 0:
                            tr, ti = tw_ref[k1:k1 + 1, :], tw_ref[N1 + k1:N1 + k1 + 1, :]
                            br, bi = br * tr + bi * ti, bi * tr - br * ti
                        fb_scr[2 * RG * k1:2 * RG * k1 + RG, :] = br
                        fb_scr[2 * RG * k1 + RG:2 * RG * (k1 + 1), :] = bi
                if ST_I <= i < ST_I + NSPL * ISTEP and (i - ST_I) % ISTEP == 0:
                    sr = RG // NSPL
                    ro = ((i - ST_I) // ISTEP) * sr
                    zs = _fft([(fb_scr[2 * RG * k1 + ro:2 * RG * k1 + ro + sr, :],
                                fb_scr[2 * RG * k1 + RG + ro:2 * RG * k1 + RG + ro + sr, :]) for k1 in range(N1)], +1)
                    for n in range(N1):
                        z_scr[pl.ds(r0 + ro, sr), 128 * n:128 * n + 128] = zs[n][0]
                        z_scr[pl.ds(LP + r0 + ro, sr), 128 * n:128 * n + 128] = zs[n][1]
        return carry

    jax.lax.fori_loop(0, H // HP, head_body, 0)

    lv = l_scr[...]
    bad = jnp.where((lv >= L_LO) & (lv <= L_HI), 0.0, 1.0)
    nbad = jnp.max(bad)

    @pl.when(nbad > 0.5)
    def _():
        TQ = 128
        def item(it, carry):
            h = it // (S // TQ)
            q0 = pl.multiple_of((it % (S // TQ)) * TQ, TQ)
            h0 = pl.multiple_of(h * 32, 32)
            qm, g0 = masked_q(h, q0, TQ, False)
            s = _nn(k_scr[:, pl.ds(g0, 128)], qm)
            m = jnp.max(s, axis=0, keepdims=True)
            p = jnp.exp2(s - m).astype(BF16)
            acc = _nn(vt_scr[pl.ds(h0, 32), :], p)
            l = acc[28:29, :]
            ot_scr[pl.ds(h0, 32), pl.ds(q0, TQ)] = (acc * (g_scr[:, pl.ds(q0, TQ)] / l)).astype(BF16)
            return carry
        jax.lax.fori_loop(0, H * (S // TQ), item, 0)

    for c in range(OCH):
        cols = slice(c * OW, (c + 1) * OW)
        zc0 = jnp.concatenate([z_scr[0:64, cols], z_scr[LP:LP + 64, cols]], axis=0).astype(BF16)
        zc2 = jnp.concatenate([z_scr[64:120, cols], z_scr[LP + 64:LP + 120, cols]], axis=0).astype(BF16)
        zc13 = jnp.concatenate([z_scr[120:176, cols], z_scr[LP + 120:LP + 176, cols],
                                z_scr[176:232, cols], z_scr[LP + 176:LP + 232, cols]], axis=0).astype(BF16)
        p0 = _nn(g02_v[0:112, :], zc0)
        p2 = _nn(g02_v[112:224, 0:112], zc2)
        ab2 = _nn(g13_v[...], zc13)
        pp, pm = p0 + p2, p0 - p2
        bt = jnp.concatenate([pp + ab2[0:112], pm + ab2[112:224], pp - ab2[0:112], pm - ab2[112:224]], axis=0)
        at = _nn(wot_scr[...], ot_scr[:, cols])
        res = at + (1.0 - g_scr[:, cols]) * bt
        out_v[:, cols] = res.astype(BF16)
        c_out[c].start()
    for c in c_out:
        c.wait()


@jax.jit
def pallas_gated_mix__softmax_full_mha__spectral_gfnet__prompt_kernel(A_x, A_wqkv, A_wo, B_x, B_w_r, B_w_i, gate_w):
    F02, F13, G02, G13, Mf, TW = _constants()
    hbm = pl.BlockSpec(memory_space=pltpu.MemorySpace.HBM)
    vmem = pl.BlockSpec(memory_space=pltpu.MemorySpace.VMEM)
    out = pl.pallas_call(
        _kernel,
        out_shape=jax.ShapeDtypeStruct((D, S), BF16),
        in_specs=[hbm, hbm, hbm, hbm, hbm, vmem, hbm, hbm, hbm, hbm, hbm, vmem],
        out_specs=hbm,
        scratch_shapes=[
            pltpu.VMEM((D, S), BF16),
            pltpu.VMEM((D, 1024), BF16),
            pltpu.VMEM((D, D), BF16),
            pltpu.VMEM((D, D), BF16),
            pltpu.VMEM((DF, S), BF16),
            pltpu.VMEM((DF, S), BF16),
            pltpu.VMEM(F02.shape, BF16),
            pltpu.VMEM(F13.shape, BF16),
            pltpu.VMEM(G02.shape, BF16),
            pltpu.VMEM(G13.shape, BF16),
            pltpu.VMEM(Mf.shape, BF16),
            pltpu.VMEM((D, S), BF16),
            pltpu.SemaphoreType.DMA((3 + XCH + 7 + OCH,)),
            pltpu.VMEM((S, 512), BF16),
            pltpu.VMEM((D + 16, S), BF16),
            pltpu.VMEM((512, S), BF16),
            pltpu.VMEM((H, S), F32),
            pltpu.VMEM((1, S), F32),
            pltpu.VMEM((H, S), F32),
            pltpu.VMEM((512, S), BF16),
            pltpu.VMEM((D, 512), BF16),
            pltpu.VMEM((2 * LP, S), F32),
            pltpu.VMEM((2 * LP, S), F32),
            pltpu.VMEM((2, S, 128), I32),
            pltpu.VMEM((N1, 256, 128), I32),
            pltpu.VMEM((N1, LP, 128), I32),
            pltpu.VMEM((N1 * 2 * RG, 128), BF16),
            pltpu.VMEM((N1 * 2 * RG, 128), F32),
            pltpu.VMEM((N1 * 2 * RG, 128), F32),
            pltpu.VMEM((SKEW + 1, KC, S), BF16),
        ],
        compiler_params=pltpu.CompilerParams(vmem_limit_bytes=110 * 1024 * 1024),
    )(A_x.reshape(S, D).T, A_wqkv, A_wo, B_w_r.T, B_w_i.T, gate_w, F02, F13, G02, G13, Mf, TW)
    return out.T.reshape(1, S, D)
```

```python
import math
import numpy as np
import jax
import jax.numpy as jnp
from jax.experimental import pallas as pl
from jax.experimental.pallas import tpu as pltpu

S, D, H, DH = 2048, 448, 16, 28
DF = D // 2 + 1
LP = 256
N1, N2 = 16, 128
QSCALE = DH ** -0.5 * math.log2(math.e)
F32, BF16, I32 = jnp.float32, jnp.bfloat16, jnp.int32
L_LO, L_HI = 2.0 ** -64, 2.0 ** 64
CLS = ((0, 0, 64, 57), (2, 64, 56, 56), (1, 120, 56, 56), (3, 176, 56, 56))
NREAL = 232


def _constants():
    d0 = np.arange(112)[None, :]

    def cs(cls, n_real, n_pad):
        l = (cls + 4 * np.arange(n_real))[:, None]
        th = 2 * np.pi * ((l * d0) % D) / D
        c = np.zeros((n_pad, 112)); s = np.zeros((n_pad, 112))
        c[:n_real] = np.cos(th); s[:n_real] = np.sin(th)
        w = np.zeros((n_pad, 1)); w[:n_real] = 2.0
        w[:n_real][(l == 0) | (l == D // 2)] = 1.0
        return c, s, w
    c0, s0, w0 = cs(0, 57, 64); c2, s2, w2 = cs(2, 56, 56); c1, s1, w1 = cs(1, 56, 56); c3, s3, w3 = cs(3, 56, 56)
    F02 = np.concatenate([c0, -s0, c2, -s2], axis=0)
    F13 = np.zeros((224, 128))
    F13[0:56, :112] = c1; F13[56:112, :112] = c3
    F13[112:168, :112] = -s1; F13[168:224, :112] = -s3
    F13[112:168, 112] = -1.0; F13[168:224, 112] = 1.0
    nrm = 1.0 / (D * S)
    G0 = np.concatenate([(w0 * c0).T, (-w0 * s0).T], axis=1) * nrm
    G2 = np.concatenate([(w2 * c2).T, (-w2 * s2).T], axis=1) * nrm
    G13 = np.zeros((240, 112))
    G13[0:112] = np.concatenate([(w1 * c1).T, (w3 * c3).T], axis=1) * nrm
    G13[112:224] = np.concatenate([(w1 * s1).T, (w3 * s3).T], axis=1) * nrm
    G13[224] = np.concatenate([-w1[:, 0], w3[:, 0]]) * nrm
    G02 = np.zeros((224, 128)); G02[:112] = G0; G02[112:, :112] = G2
    n2 = np.arange(N2)[:, None]; k2 = np.arange(N2)[None, :]
    th = 2 * np.pi * ((n2 * k2) % N2) / N2
    Fr, Fi = np.cos(th), -np.sin(th)
    FF = np.where(n2 <= N2 // 2, np.cos(th), np.sin(th))
    FF[0] *= 0.5; FF[N2 // 2] *= 0.5
    k1 = np.arange(N1)[:, None]
    tt = 2 * np.pi * ((k1 * np.arange(N2)[None, :]) % S) / S
    TW = np.concatenate([np.cos(tt), -np.sin(tt)], axis=0)
    return tuple(jnp.asarray(m, BF16) for m in (F02, F13, G02, G13, FF)) + (jnp.asarray(TW, F32),)


def _cmul_const(re, im, k, n, sign):
    k = k % n
    if k == 0:
        return re, im
    if 4 * k == n:
        return (-im, re) if sign > 0 else (im, -re)
    if 2 * k == n:
        return -re, -im
    if 4 * k == 3 * n:
        return (im, -re) if sign > 0 else (-im, re)
    c = math.cos(2 * math.pi * k / n); s = sign * math.sin(2 * math.pi * k / n)
    if (8 * k) % n == 0:
        a = abs(c)
        sc, ss = (1 if c > 0 else -1), (1 if s > 0 else -1)
        rr = (re - im) if sc == ss else (re + im)
        ii = (re + im) if sc == ss else (im - re)
        return rr * (sc * a), ii * (sc * a)
    return re * c - im * s, re * s + im * c


def _fft(xs, sign):
    n = len(xs)
    if n == 1:
        return xs
    ev = _fft(xs[0::2], sign)
    od = _fft(xs[1::2], sign)
    out = [None] * n
    for k in range(n // 2):
        tr, ti = _cmul_const(od[k][0], od[k][1], k, n, sign)
        out[k] = (ev[k][0] + tr, ev[k][1] + ti)
        out[k + n // 2] = (ev[k][0] - tr, ev[k][1] - ti)
    return out


def _nt(a, b):
    return jax.lax.dot_general(a, b, (((1,), (1,)), ((), ())), preferred_element_type=F32)


def _nn(a, b):
    return jnp.dot(a, b, preferred_element_type=F32)


def _rev(x):
    lane = jax.lax.broadcasted_iota(I32, x.shape, 1)
    return jnp.take_along_axis(x, (N2 - lane) % N2, axis=1)


def _reflect(y):
    sub = jax.lax.broadcasted_iota(I32, (8, y.shape[1]), 0)
    idx = (8 - sub) % 8
    g = [jnp.take_along_axis(y[8 * j:8 * j + 8], idx, axis=0) for j in range(15)]
    return jnp.concatenate([jnp.where(sub == 0, g[14 - j], g[13 - j]) for j in range(14)], axis=0)


def _fold(re, im, sign):
    lane = jax.lax.broadcasted_iota(I32, re.shape, 1)
    lo = lane <= N2 // 2
    rr, ri = _rev(re), _rev(im)
    if sign < 0:
        return jnp.where(lo, re + rr, im - ri), jnp.where(lo, im + ri, rr - re)
    return jnp.where(lo, re + rr, ri - im), jnp.where(lo, im + ri, re - rr)


KC = 128
PEXP = 1
SKEW = 2
HP = 2
RG = LP // (H // HP)
KP = 1
NP = N1 // KP
NSPL = 2
ISTEP = 2
BPOS = 0
DLEAD = 1
NSG = 4
ST_X = 1
ST_Y = 6
ST_I = 0
XCH = 4
XW = S // XCH
OCH = 8
OW = S // OCH


def _kernel(xa_hbm, wqkv_hbm, wo_hbm, wr_hbm, wi_hbm, gw_ref, f02_hbm, f13_hbm, g02_hbm, g13_hbm, mf_hbm, tw_ref,
            out_hbm,
            x_v, wq_v, wk_v, wv_v, wo_v, wr_v, wi_v, f02_v, f13_v, g02_v, g13_v, mf_v, out_v, sems,
            k_scr, qt_scr, vt_scr, negm_scr, g_scr, l_scr, ot_scr,
            u_scr, c_scr, wn_scr, wp_scr, wc_scr, fa_scr, fb_scr, p_scr):
    nsem = [0]

    def cp(src, dst):
        nsem[0] += 1
        return pltpu.make_async_copy(src, dst, sems.at[nsem[0] - 1])

    c_wq = cp(wqkv_hbm.at[:, pl.ds(0, 512)], wq_v)
    c_wk = cp(wqkv_hbm.at[:, pl.ds(384, 640)], wk_v)
    c_f = [cp(f02_hbm, f02_v), cp(f13_hbm, f13_v)]
    c_x = [cp(xa_hbm.at[:, pl.ds(c * XW, XW)], x_v.at[:, pl.ds(c * XW, XW)]) for c in range(XCH)]
    rest = [cp(wqkv_hbm.at[:, pl.ds(896, 448)], wv_v), cp(wr_hbm, wr_v), cp(wi_hbm, wi_v), cp(mf_hbm, mf_v),
            cp(wo_hbm, wo_v), cp(g02_hbm, g02_v), cp(g13_hbm, g13_v)]
    c_out = [cp(out_v.at[:, pl.ds(c * OW, OW)], out_hbm.at[:, pl.ds(c * OW, OW)]) for c in range(OCH)]
    c_wq.start()
    c_x[0].start()
    c_wq.wait()
    c_wk.start()
    for c in c_f:
        c.start()
    for c in c_x[1:]:
        c.start()

    wqT = jnp.concatenate([wq_v[...].astype(F32).T[0:D, :], gw_ref[...].astype(F32).reshape(1, D),
                           jnp.zeros((15, D), F32)], axis=0).astype(BF16)
    w_box = {}

    lane = jax.lax.broadcasted_iota(I32, (XW, 128), 1)
    kmax = [None] * 4

    def dfwd_prep(c):
        cols = slice(c * XW, (c + 1) * XW)
        xf = x_v[:, cols].astype(F32)
        x0, x1, x2, x3 = (xf[112 * j:112 * j + 112] for j in range(4))
        s02, s13 = x0 + x2, x1 + x3
        e0 = (s02 + s13).astype(BF16)
        e2 = (s02 - s13).astype(BF16)
        a, b = x0 - x2, x1 - x3
        bt = _reflect(jnp.concatenate([b, jnp.zeros((8, XW), F32)], axis=0))
        pp = (a - bt).astype(BF16)
        mm = jnp.concatenate([a + bt, b[0:1], jnp.zeros((15, XW), F32)], axis=0).astype(BF16)
        return e0, e2, pp, mm

    def dfwd_mm(c, ops):
        cols = slice(c * XW, (c + 1) * XW)
        e0, e2, pp, mm = ops
        r0 = _nn(f02_v[0:128, :], e0)
        r2 = _nn(f02_v[128:240, :], e2)
        rc = _nn(f13_v[0:112, 0:112], pp)
        rs = _nn(f13_v[112:224, :], mm)
        zpad = jnp.zeros((LP - NREAL, XW), F32)
        u_scr[0:LP, cols] = jnp.concatenate([r0[0:64], r2[0:56], rc, zpad], axis=0)
        u_scr[LP:2 * LP, cols] = jnp.concatenate([r0[64:128], r2[56:112], rs, zpad], axis=0)

    def dfwd(c):
        dfwd_mm(c, dfwd_prep(c))

    def qproj(c):
        cols = slice(c * XW, (c + 1) * XW)
        qf = _nn(wqT, x_v[:, cols])
        g_scr[:, cols] = jax.nn.sigmoid(qf[D:D + 1, :])
        qt_scr[:, cols] = (qf * QSCALE).astype(BF16)

    def kproj(c):
        cols = slice(c * XW, (c + 1) * XW)
        kt = _nn(w_box["k"], x_v[:, cols])
        zr = jnp.zeros((16, XW), F32)
        for g in range(4):
            kg = kt[112 * g: 112 * g + 128, :] if g < 3 else jnp.concatenate([kt[336:448, :], zr], axis=0)
            kg = jnp.where(lane == 112, 1.0, kg.T)
            k_scr[cols, 128 * g:128 * g + 128] = kg.astype(BF16)
            km = jnp.max(jnp.abs(kg), axis=0, keepdims=True)
            kmax[g] = km if kmax[g] is None else jnp.maximum(kmax[g], km)

    def qkproj(c):
        qproj(c)
        kproj(c)

    def wshuf_first():
        wrb = pltpu.bitcast(wr_v[...].astype(F32), I32)
        wib = pltpu.bitcast(wi_v[...].astype(F32), I32)
        wpk = wrb | jax.lax.shift_right_logical(wib, 16)
        wpk = jnp.concatenate([wpk, jnp.zeros((256 - DF, S), I32)], axis=0)
        wn = wpk.T
        wn_scr[0] = wn[:, 0:128]
        wn_scr[1] = wn[:, 128:256]

    def wshuf_second(k1):
        for t in range(2):
            wp_scr[k1, 128 * t:128 * t + 128, :] = wn_scr[t, pl.ds(k1, N2, stride=N1), :].T
        wc_scr[k1] = jnp.concatenate([wp_scr[k1, pl.ds(c, n, stride=4), :] for c, _, n, _ in CLS]
                                     + [jnp.zeros((LP - NREAL, 128), I32)], axis=0)

    c_x[0].wait()
    qproj(0)
    c_wk.wait()
    for cf in c_f:
        cf.wait()
    for cr in rest:
        cr.start()
    w_box["k"] = wk_v[...].astype(F32).T[64:64 + D, :].astype(BF16)
    dfwd(0)
    kproj(0)
    for c in range(1, XCH):
        c_x[c].wait()
    for c in range(1, XCH - 1):
        qkproj(c)
        dfwd(c)

    for cr in rest:
        cr.wait()

    qkproj(XCH - 1)
    dfwd(XCH - 1)
    wvT = wv_v[...].astype(F32).T.astype(BF16)
    wshuf_first()

    def bound():
        hh = jax.lax.broadcasted_iota(I32, (8, 128), 0)
        ll = jax.lax.broadcasted_iota(I32, (8, 128), 1)
        for g in range(4):
            ind = jnp.where((ll >= hh * DH) & (ll < hh * DH + DH) & (hh < 4), kmax[g] * 1.02, 0.0).astype(BF16)
            qa = pltpu.bitcast(pltpu.bitcast(qt_scr[112 * g:112 * g + 128, :], I32) & jnp.int32(0x7FFF7FFF), BF16)
            mt = _nn(ind, qa)
            negm_scr[4 * g:4 * g + 4, :] = -mt[0:4]

    tail_rows = jnp.concatenate([jnp.ones((1, XW), F32), jnp.zeros((3, XW), F32)], axis=0)
    for c in range(XCH):
        cols = slice(c * XW, (c + 1) * XW)
        vt = _nn(wvT, x_v[:, cols])
        for h in range(H):
            vt_scr[32 * h:32 * h + 32, cols] = jnp.concatenate(
                [vt[DH * h:DH * h + DH, :], tail_rows], axis=0).astype(BF16)
        for k1 in range(4 * c, 4 * c + 4):
            wshuf_second(k1)
        if c == BPOS:
            bound()

    def masked_q(h, q0, tq, with_shift):
        g = h // 4
        r0 = pl.multiple_of(g * 112, 16)
        g0 = pl.multiple_of(g * 128, 128)
        j0 = (h % 4) * DH
        qs = qt_scr[pl.ds(r0, 128), pl.ds(q0, tq)]
        rows = jax.lax.broadcasted_iota(I32, (128, tq), 0)
        qm = jnp.where((rows >= j0) & (rows < j0 + DH), qs.astype(F32), 0.0)
        if with_shift:
            qm = jnp.where(rows == 112, negm_scr[pl.ds(h, 1), pl.ds(q0, tq)], qm)
        return qm.astype(BF16), g0

    FX0 = N1 * 2 * LP
    SR = RG // NSG
    PR = N1 * 2 * SR

    def fwd_stage(r0, j):
        ro = j * SR
        xs = [(u_scr[pl.ds(r0 + ro, SR), 128 * n:128 * n + 128],
               u_scr[pl.ds(LP + r0 + ro, SR), 128 * n:128 * n + 128]) for n in range(N1)]
        ys = _fft(xs, -1)
        for k1 in range(N1):
            ar, ai = ys[k1]
            if k1 > 0:
                tr, ti = tw_ref[k1:k1 + 1, :], tw_ref[N1 + k1:N1 + k1 + 1, :]
                ar, ai = ar * tr - ai * ti, ar * ti + ai * tr
            f1, f2 = _fold(ar, ai, -1)
            fa_scr[2 * SR * k1:2 * SR * (k1 + 1), :] = jnp.concatenate([f1, f2], axis=0).astype(BF16)

    def x_stage():
        c_scr[FX0:FX0 + PR, :] = _nn(fa_scr[0:PR, :], mf_v[...])

    def y_stage(r0, j):
        ro = j * SR
        ys_ = []
        for k1 in range(N1):
            xr = c_scr[FX0 + 2 * SR * k1:FX0 + 2 * SR * k1 + SR, :]
            xi = c_scr[FX0 + 2 * SR * k1 + SR:FX0 + 2 * SR * (k1 + 1), :]
            w = wc_scr[k1, pl.ds(r0 + ro, SR), :]
            wr = pltpu.bitcast(w & jnp.int32(-65536), F32)
            wi = pltpu.bitcast(jax.lax.shift_left(w, 16), F32)
            ys_ += list(_fold(xr * wr - xi * wi, xr * wi + xi * wr, +1))
        fb_scr[0:PR, :] = _nn(jnp.concatenate(ys_, axis=0).astype(BF16), mf_v[...])

    def inv_stage(r0, j):
        ro = j * SR
        bs = []
        for k1 in range(N1):
            br = fb_scr[2 * SR * k1:2 * SR * k1 + SR, :]
            bi = fb_scr[2 * SR * k1 + SR:2 * SR * (k1 + 1), :]
            if k1 > 0:
                tr, ti = tw_ref[k1:k1 + 1, :], tw_ref[N1 + k1:N1 + k1 + 1, :]
                br, bi = br * tr + bi * ti, bi * tr - br * ti
            bs.append((br, bi))
        zs = _fft(bs, +1)
        for n in range(N1):
            c_scr[pl.ds(2 * LP * n + r0 + ro, SR), :] = zs[n][0]
            c_scr[pl.ds(2 * LP * n + LP + r0 + ro, SR), :] = zs[n][1]

    def head_body(t, carry):
        nc = S // KC
        seq = [(u, c) for u in range(HP) for c in range(nc)]
        qms = {}
        accs = {}
        r0 = pl.multiple_of(t * RG, 8)
        rp = pl.multiple_of(((t + H // HP - 1) % (H // HP)) * RG, 8)
        per = len(seq) // NSG
        for i in range(len(seq) + SKEW):
            j, ph = divmod(i, per)
            if j < NSG and ph == ST_X:
                if j == 0:
                    inv_stage(rp, NSG - 1)
                else:
                    inv_stage(r0, j - 1)
                fwd_stage(r0, j)
            if i < len(seq):
                u, c = seq[i]
                h = HP * t + u
                if c == 0:
                    qms[u] = masked_q(h, 0, S, True)
                qm, g0 = qms[u]
                s = _nn(k_scr[pl.ds(c * KC, KC), pl.ds(g0, 128)], qm)
                p_scr[i % (SKEW + 1)] = jnp.exp2(s).astype(BF16)
            if i >= SKEW:
                u, c = seq[i - SKEW]
                h = HP * t + u
                h0 = pl.multiple_of(h * 32, 32)
                ov = _nn(vt_scr[pl.ds(h0, 32), pl.ds(c * KC, KC)], p_scr[(i - SKEW) % (SKEW + 1)])
                accs[u] = ov if u not in accs else accs[u] + ov
                if c == nc - 1:
                    acc = accs[u]
                    l = acc[28:29, :]
                    l_scr[pl.ds(h, 1), :] = l
                    ot_scr[pl.ds(h0, 32), :] = (acc * (g_scr[...] / l)).astype(BF16)
            if j < NSG and ph == ST_X:
                x_stage()
            if j < NSG and ph == ST_Y:
                y_stage(r0, j)
        return carry

    fb_scr[...] = jnp.zeros(fb_scr.shape, F32)
    jax.lax.fori_loop(0, H // HP, head_body, 0)

    lv = l_scr[...]
    bad = jnp.where((lv >= L_LO) & (lv <= L_HI), 0.0, 1.0)
    nbad = jnp.max(bad)

    @pl.when(nbad > 0.5)
    def _():
        TQ = 128
        def item(it, carry):
            h = it // (S // TQ)
            q0 = pl.multiple_of((it % (S // TQ)) * TQ, TQ)
            h0 = pl.multiple_of(h * 32, 32)
            qm, g0 = masked_q(h, q0, TQ, False)
            s = _nn(k_scr[:, pl.ds(g0, 128)], qm)
            m = jnp.max(s, axis=0, keepdims=True)
            p = jnp.exp2(s - m).astype(BF16)
            acc = _nn(vt_scr[pl.ds(h0, 32), :], p)
            l = acc[28:29, :]
            ot_scr[pl.ds(h0, 32), pl.ds(q0, TQ)] = (acc * (g_scr[:, pl.ds(q0, TQ)] / l)).astype(BF16)
            return carry
        jax.lax.fori_loop(0, H * (S // TQ), item, 0)

    def zrows(a, b, c):
        nt = OW // 128
        return jnp.concatenate([c_scr[2 * LP * n + a:2 * LP * n + b, :] for n in range(c * nt, (c + 1) * nt)], axis=1)

    z4 = jnp.zeros((4, D), F32)

    def dinv(c):
        zc0 = jnp.concatenate([zrows(0, 64, c), zrows(LP, LP + 64, c)], axis=0).astype(BF16)
        zc2 = jnp.concatenate([zrows(64, 120, c), zrows(LP + 64, LP + 120, c)], axis=0).astype(BF16)
        zr13 = zrows(120, 232, c).astype(BF16)
        zi13 = zrows(LP + 120, LP + 232, c).astype(BF16)
        p0 = _nn(g02_v[0:112, :], zc0)
        p2 = _nn(g02_v[112:224, 0:112], zc2)
        pc = _nn(g13_v[0:112, :], zr13)
        qs = _nn(g13_v[112:240, :], zi13)
        aa = pc - qs[0:112]
        bb = _reflect(jnp.concatenate([-(pc + qs[0:112]), qs[112:120]], axis=0))
        pp, pm = p0 + p2, p0 - p2
        return jnp.concatenate([pp + aa, pm + bb, pp - aa, pm - bb], axis=0)

    wo = wo_v[...].astype(F32)
    parts = []
    for h in range(H):
        parts += [wo[DH * h: DH * h + DH, :], z4]
    wo_pad = jnp.concatenate(parts, axis=0)
    woT = jnp.concatenate([wo_pad, jnp.zeros((512, 64), F32)], axis=1).T[:D, :].astype(BF16)
    bts = {c: dinv(c) for c in range(DLEAD)}
    for c in range(OCH):
        cols = slice(c * OW, (c + 1) * OW)
        if c + DLEAD < OCH:
            bts[c + DLEAD] = dinv(c + DLEAD)
        at = _nn(woT, ot_scr[:, cols])
        res = at + (1.0 - g_scr[:, cols]) * bts.pop(c)
        out_v[:, cols] = res.astype(BF16)
        c_out[c].start()
    for c in c_out:
        c.wait()


@jax.jit
def pallas_gated_mix__softmax_full_mha__spectral_gfnet__prompt_kernel(A_x, A_wqkv, A_wo, B_x, B_w_r, B_w_i, gate_w):
    F02, F13, G02, G13, Mf, TW = _constants()
    hbm = pl.BlockSpec(memory_space=pltpu.MemorySpace.HBM)
    vmem = pl.BlockSpec(memory_space=pltpu.MemorySpace.VMEM)
    out = pl.pallas_call(
        _kernel,
        out_shape=jax.ShapeDtypeStruct((D, S), BF16),
        in_specs=[hbm, hbm, hbm, hbm, hbm, vmem, hbm, hbm, hbm, hbm, hbm, vmem],
        out_specs=hbm,
        scratch_shapes=[
            pltpu.VMEM((D, S), BF16),
            pltpu.VMEM((D, 512), BF16),
            pltpu.VMEM((D, 640), BF16),
            pltpu.VMEM((D, D), BF16),
            pltpu.VMEM((D, D), BF16),
            pltpu.VMEM((DF, S), BF16),
            pltpu.VMEM((DF, S), BF16),
            pltpu.VMEM(F02.shape, BF16),
            pltpu.VMEM(F13.shape, BF16),
            pltpu.VMEM(G02.shape, BF16),
            pltpu.VMEM(G13.shape, BF16),
            pltpu.VMEM(Mf.shape, BF16),
            pltpu.VMEM((D, S), BF16),
            pltpu.SemaphoreType.DMA((4 + XCH + 7 + OCH,)),
            pltpu.VMEM((S, 512), BF16),
            pltpu.VMEM((D + 16, S), BF16),
            pltpu.VMEM((512, S), BF16),
            pltpu.VMEM((H, S), F32),
            pltpu.VMEM((1, S), F32),
            pltpu.VMEM((H, S), F32),
            pltpu.VMEM((512, S), BF16),
            pltpu.VMEM((2 * LP, S), F32),
            pltpu.VMEM((N1 * 2 * LP + N1 * 2 * RG, 128), F32),
            pltpu.VMEM((2, S, 128), I32),
            pltpu.VMEM((N1, 256, 128), I32),
            pltpu.VMEM((N1, LP, 128), I32),
            pltpu.VMEM((N1 * 2 * RG, 128), BF16),
            pltpu.VMEM((N1 * 2 * RG, 128), F32),
            pltpu.VMEM((SKEW + 1, KC, S), BF16),
        ],
        compiler_params=pltpu.CompilerParams(vmem_limit_bytes=110 * 1024 * 1024),
    )(A_x.reshape(S, D).T, A_wqkv, A_wo, B_w_r.T, B_w_i.T, gate_w, F02, F13, G02, G13, Mf, TW)
    return out.T.reshape(1, S, D)
```

```python
import math
import numpy as np
import jax
import jax.numpy as jnp
from jax.experimental import pallas as pl
from jax.experimental.pallas import tpu as pltpu

S, D, H, DH = 2048, 448, 16, 28
DF = D // 2 + 1
LP = 256
N1, N2 = 16, 128
QSCALE = DH ** -0.5 * math.log2(math.e)
F32, BF16, I32 = jnp.float32, jnp.bfloat16, jnp.int32
L_LO, L_HI = 2.0 ** -64, 2.0 ** 64
CLS = ((0, 0, 64, 57), (2, 64, 56, 56), (1, 120, 56, 56), (3, 176, 56, 56))
NREAL = 232


def _constants():
    d0 = np.arange(112)[None, :]

    def cs(cls, n_real, n_pad):
        l = (cls + 4 * np.arange(n_real))[:, None]
        th = 2 * np.pi * ((l * d0) % D) / D
        c = np.zeros((n_pad, 112)); s = np.zeros((n_pad, 112))
        c[:n_real] = np.cos(th); s[:n_real] = np.sin(th)
        w = np.zeros((n_pad, 1)); w[:n_real] = 2.0
        w[:n_real][(l == 0) | (l == D // 2)] = 1.0
        return c, s, w
    c0, s0, w0 = cs(0, 57, 64); c2, s2, w2 = cs(2, 56, 56); c1, s1, w1 = cs(1, 56, 56); c3, s3, w3 = cs(3, 56, 56)
    F02 = np.concatenate([c0, -s0, c2, -s2], axis=0)
    F13 = np.zeros((224, 128))
    F13[0:56, :112] = c1; F13[56:112, :112] = c3
    F13[112:168, :112] = -s1; F13[168:224, :112] = -s3
    F13[112:168, 112] = -1.0; F13[168:224, 112] = 1.0
    nrm = 1.0 / (D * S)
    G0 = np.concatenate([(w0 * c0).T, (-w0 * s0).T], axis=1) * nrm
    G2 = np.concatenate([(w2 * c2).T, (-w2 * s2).T], axis=1) * nrm
    G13 = np.zeros((240, 112))
    G13[0:112] = np.concatenate([(w1 * c1).T, (w3 * c3).T], axis=1) * nrm
    G13[112:224] = np.concatenate([(w1 * s1).T, (w3 * s3).T], axis=1) * nrm
    G13[224] = np.concatenate([-w1[:, 0], w3[:, 0]]) * nrm
    G02 = np.zeros((224, 128)); G02[:112] = G0; G02[112:, :112] = G2
    n2 = np.arange(N2)[:, None]; k2 = np.arange(N2)[None, :]
    th = 2 * np.pi * ((n2 * k2) % N2) / N2
    Fr, Fi = np.cos(th), -np.sin(th)
    FF = np.where(n2 <= N2 // 2, np.cos(th), np.sin(th))
    FF[0] *= 0.5; FF[N2 // 2] *= 0.5
    k1 = np.arange(N1)[:, None]
    tt = 2 * np.pi * ((k1 * np.arange(N2)[None, :]) % S) / S
    TW = np.concatenate([np.cos(tt), -np.sin(tt)], axis=0)
    return tuple(jnp.asarray(m, BF16) for m in (F02, F13, G02, G13, FF)) + (jnp.asarray(TW, F32),)


def _cmul_const(re, im, k, n, sign):
    k = k % n
    if k == 0:
        return re, im
    if 4 * k == n:
        return (-im, re) if sign > 0 else (im, -re)
    if 2 * k == n:
        return -re, -im
    if 4 * k == 3 * n:
        return (im, -re) if sign > 0 else (-im, re)
    c = math.cos(2 * math.pi * k / n); s = sign * math.sin(2 * math.pi * k / n)
    if (8 * k) % n == 0:
        a = abs(c)
        sc, ss = (1 if c > 0 else -1), (1 if s > 0 else -1)
        rr = (re - im) if sc == ss else (re + im)
        ii = (re + im) if sc == ss else (im - re)
        return rr * (sc * a), ii * (sc * a)
    return re * c - im * s, re * s + im * c


def _fft(xs, sign):
    n = len(xs)
    if n == 1:
        return xs
    ev = _fft(xs[0::2], sign)
    od = _fft(xs[1::2], sign)
    out = [None] * n
    for k in range(n // 2):
        tr, ti = _cmul_const(od[k][0], od[k][1], k, n, sign)
        out[k] = (ev[k][0] + tr, ev[k][1] + ti)
        out[k + n // 2] = (ev[k][0] - tr, ev[k][1] - ti)
    return out


def _nt(a, b):
    return jax.lax.dot_general(a, b, (((1,), (1,)), ((), ())), preferred_element_type=F32)


def _nn(a, b):
    return jnp.dot(a, b, preferred_element_type=F32)


def _rev(x):
    lane = jax.lax.broadcasted_iota(I32, x.shape, 1)
    return jnp.take_along_axis(x, (N2 - lane) % N2, axis=1)


def _reflect(y):
    sub = jax.lax.broadcasted_iota(I32, (8, y.shape[1]), 0)
    idx = (8 - sub) % 8
    g = [jnp.take_along_axis(y[8 * j:8 * j + 8], idx, axis=0) for j in range(15)]
    return jnp.concatenate([jnp.where(sub == 0, g[14 - j], g[13 - j]) for j in range(14)], axis=0)


def _fold(re, im, sign):
    lane = jax.lax.broadcasted_iota(I32, re.shape, 1)
    lo = lane <= N2 // 2
    rr, ri = _rev(re), _rev(im)
    if sign < 0:
        return jnp.where(lo, re + rr, im - ri), jnp.where(lo, im + ri, rr - re)
    return jnp.where(lo, re + rr, ri - im), jnp.where(lo, im + ri, re - rr)


KC = 256
PEXP = 1
SKEW = 1
HP = 2
RG = LP // (H // HP)
KP = 1
NP = N1 // KP
NSPL = 2
ISTEP = 2
BPOS = 3
DLEAD = 1
NSG = 4
ST_X = 0
ST_Y = 3
ST_I = 0
XCH = 4
XW = S // XCH
OCH = 16
OW = S // OCH


def _kernel(xa_hbm, wqkv_hbm, wo_hbm, wr_hbm, wi_hbm, gw_ref, f02_hbm, f13_hbm, g02_hbm, g13_hbm, mf_hbm, tw_ref,
            out_hbm,
            x_v, wq_v, wk_v, wv_v, wo_v, wr_v, wi_v, f02_v, f13_v, g02_v, g13_v, mf_v, out_v, sems,
            k_scr, qt_scr, vt_scr, negm_scr, g_scr, l_scr, ot_scr,
            u_scr, c_scr, wn_scr, wp_scr, wc_scr, fa_scr, fb_scr, p_scr):
    nsem = [0]

    def cp(src, dst):
        nsem[0] += 1
        return pltpu.make_async_copy(src, dst, sems.at[nsem[0] - 1])

    c_wq = cp(wqkv_hbm.at[:, pl.ds(0, 512)], wq_v)
    c_wk = cp(wqkv_hbm.at[:, pl.ds(384, 640)], wk_v)
    c_f = [cp(f02_hbm, f02_v), cp(f13_hbm, f13_v)]
    c_x = [cp(xa_hbm.at[:, pl.ds(c * XW, XW)], x_v.at[:, pl.ds(c * XW, XW)]) for c in range(XCH)]
    rest = [cp(wqkv_hbm.at[:, pl.ds(896, 448)], wv_v), cp(wr_hbm, wr_v), cp(wi_hbm, wi_v), cp(mf_hbm, mf_v),
            cp(wo_hbm, wo_v), cp(g02_hbm, g02_v), cp(g13_hbm, g13_v)]
    c_out = [cp(out_v.at[:, pl.ds(c * OW, OW)], out_hbm.at[:, pl.ds(c * OW, OW)]) for c in range(OCH)]
    c_wq.start()
    c_x[0].start()
    c_wq.wait()
    c_wk.start()
    for c in c_f:
        c.start()
    for c in c_x[1:]:
        c.start()

    wqT = jnp.concatenate([wq_v[...].astype(F32).T[0:D, :], gw_ref[...].astype(F32).reshape(1, D),
                           jnp.zeros((15, D), F32)], axis=0).astype(BF16)
    w_box = {}

    lane = jax.lax.broadcasted_iota(I32, (XW, 128), 1)
    kmax = [None] * 4

    def dfwd_prep(c):
        cols = slice(c * XW, (c + 1) * XW)
        xf = x_v[:, cols].astype(F32)
        x0, x1, x2, x3 = (xf[112 * j:112 * j + 112] for j in range(4))
        s02, s13 = x0 + x2, x1 + x3
        e0 = (s02 + s13).astype(BF16)
        e2 = (s02 - s13).astype(BF16)
        a, b = x0 - x2, x1 - x3
        bt = _reflect(jnp.concatenate([b, jnp.zeros((8, XW), F32)], axis=0))
        pp = (a - bt).astype(BF16)
        mm = jnp.concatenate([a + bt, b[0:1], jnp.zeros((15, XW), F32)], axis=0).astype(BF16)
        return e0, e2, pp, mm

    def dfwd_mm(c, ops):
        cols = slice(c * XW, (c + 1) * XW)
        e0, e2, pp, mm = ops
        r0 = _nn(f02_v[0:128, :], e0)
        r2 = _nn(f02_v[128:240, :], e2)
        rc = _nn(f13_v[0:112, 0:112], pp)
        rs = _nn(f13_v[112:224, :], mm)
        zpad = jnp.zeros((LP - NREAL, XW), F32)
        u_scr[0:LP, cols] = jnp.concatenate([r0[0:64], r2[0:56], rc, zpad], axis=0)
        u_scr[LP:2 * LP, cols] = jnp.concatenate([r0[64:128], r2[56:112], rs, zpad], axis=0)

    def dfwd(c):
        dfwd_mm(c, dfwd_prep(c))

    def qproj(c):
        cols = slice(c * XW, (c + 1) * XW)
        qf = _nn(wqT, x_v[:, cols])
        g_scr[:, cols] = jax.nn.sigmoid(qf[D:D + 1, :])
        qt_scr[:, cols] = (qf * QSCALE).astype(BF16)

    def kproj(c):
        cols = slice(c * XW, (c + 1) * XW)
        kt = _nn(w_box["k"], x_v[:, cols])
        zr = jnp.zeros((16, XW), F32)
        for g in range(4):
            kg = kt[112 * g: 112 * g + 128, :] if g < 3 else jnp.concatenate([kt[336:448, :], zr], axis=0)
            kg = jnp.where(lane == 112, 1.0, kg.T)
            k_scr[cols, 128 * g:128 * g + 128] = kg.astype(BF16)
            km = jnp.max(jnp.abs(kg), axis=0, keepdims=True)
            kmax[g] = km if kmax[g] is None else jnp.maximum(kmax[g], km)

    def qkproj(c):
        qproj(c)
        kproj(c)

    def wshuf_first():
        wrb = pltpu.bitcast(wr_v[...].astype(F32), I32)
        wib = pltpu.bitcast(wi_v[...].astype(F32), I32)
        wpk = wrb | jax.lax.shift_right_logical(wib, 16)
        wpk = jnp.concatenate([wpk, jnp.zeros((256 - DF, S), I32)], axis=0)
        wn = wpk.T
        wn_scr[0] = wn[:, 0:128]
        wn_scr[1] = wn[:, 128:256]

    def wshuf_second(k1):
        for t in range(2):
            wp_scr[k1, 128 * t:128 * t + 128, :] = wn_scr[t, pl.ds(k1, N2, stride=N1), :].T
        wc_scr[k1] = jnp.concatenate([wp_scr[k1, pl.ds(c, n, stride=4), :] for c, _, n, _ in CLS]
                                     + [jnp.zeros((LP - NREAL, 128), I32)], axis=0)

    c_x[0].wait()
    qproj(0)
    c_wk.wait()
    for cf in c_f:
        cf.wait()
    for cr in rest:
        cr.start()
    w_box["k"] = wk_v[...].astype(F32).T[64:64 + D, :].astype(BF16)
    dfwd(0)
    kproj(0)
    for c in range(1, XCH):
        c_x[c].wait()
    for c in range(1, XCH - 1):
        qkproj(c)
        dfwd(c)

    for cr in rest:
        cr.wait()

    qkproj(XCH - 1)
    dfwd(XCH - 1)
    wvT = wv_v[...].astype(F32).T.astype(BF16)
    wshuf_first()

    def bound():
        hh = jax.lax.broadcasted_iota(I32, (8, 128), 0)
        ll = jax.lax.broadcasted_iota(I32, (8, 128), 1)
        for g in range(4):
            ind = jnp.where((ll >= hh * DH) & (ll < hh * DH + DH) & (hh < 4), kmax[g] * 1.02, 0.0).astype(BF16)
            qa = pltpu.bitcast(pltpu.bitcast(qt_scr[112 * g:112 * g + 128, :], I32) & jnp.int32(0x7FFF7FFF), BF16)
            mt = _nn(ind, qa)
            negm_scr[4 * g:4 * g + 4, :] = -mt[0:4]

    tail_rows = jnp.concatenate([jnp.ones((1, XW), F32), jnp.zeros((3, XW), F32)], axis=0)
    for c in range(XCH):
        cols = slice(c * XW, (c + 1) * XW)
        vt = _nn(wvT, x_v[:, cols])
        for h in range(H):
            vt_scr[32 * h:32 * h + 32, cols] = jnp.concatenate(
                [vt[DH * h:DH * h + DH, :], tail_rows], axis=0).astype(BF16)
        for k1 in range(4 * c, 4 * c + 4):
            wshuf_second(k1)
        if c == BPOS:
            bound()

    def masked_q(h, q0, tq, with_shift):
        g = h // 4
        r0 = pl.multiple_of(g * 112, 16)
        g0 = pl.multiple_of(g * 128, 128)
        w0 = (h % 4) * (DH // 2)
        qw = pltpu.bitcast(qt_scr[pl.ds(r0, 128), pl.ds(q0, tq)], I32)
        rows = jax.lax.broadcasted_iota(I32, (64, tq), 0)
        qm = jnp.where((rows >= w0) & (rows < w0 + DH // 2), qw, 0)
        if with_shift:
            sh = negm_scr[pl.ds(h, 1), pl.ds(q0, tq)].astype(BF16).astype(F32)
            shw = jax.lax.shift_right_logical(pltpu.bitcast(sh, I32), 16)
            qm = jnp.where(rows == 56, shw, qm)
        return pltpu.bitcast(qm, BF16), g0

    FX0 = N1 * 2 * LP
    SR = RG // NSG
    PR = N1 * 2 * SR

    def fwd_stage(r0, j):
        ro = j * SR
        xs = [(u_scr[pl.ds(r0 + ro, SR), 128 * n:128 * n + 128],
               u_scr[pl.ds(LP + r0 + ro, SR), 128 * n:128 * n + 128]) for n in range(N1)]
        ys = _fft(xs, -1)
        for k1 in range(N1):
            ar, ai = ys[k1]
            if k1 > 0:
                tr, ti = tw_ref[k1:k1 + 1, :], tw_ref[N1 + k1:N1 + k1 + 1, :]
                ar, ai = ar * tr - ai * ti, ar * ti + ai * tr
            f1, f2 = _fold(ar, ai, -1)
            fa_scr[2 * SR * k1:2 * SR * (k1 + 1), :] = jnp.concatenate([f1, f2], axis=0).astype(BF16)

    def x_stage():
        c_scr[FX0:FX0 + PR, :] = _nn(fa_scr[0:PR, :], mf_v[...])

    def y_stage(r0, j):
        ro = j * SR
        ys_ = []
        for k1 in range(N1):
            xr = c_scr[FX0 + 2 * SR * k1:FX0 + 2 * SR * k1 + SR, :]
            xi = c_scr[FX0 + 2 * SR * k1 + SR:FX0 + 2 * SR * (k1 + 1), :]
            w = wc_scr[k1, pl.ds(r0 + ro, SR), :]
            wr = pltpu.bitcast(w & jnp.int32(-65536), F32)
            wi = pltpu.bitcast(jax.lax.shift_left(w, 16), F32)
            ys_ += list(_fold(xr * wr - xi * wi, xr * wi + xi * wr, +1))
        fb_scr[0:PR, :] = _nn(jnp.concatenate(ys_, axis=0).astype(BF16), mf_v[...])

    def inv_stage(r0, j):
        ro = j * SR
        bs = []
        for k1 in range(N1):
            br = fb_scr[2 * SR * k1:2 * SR * k1 + SR, :]
            bi = fb_scr[2 * SR * k1 + SR:2 * SR * (k1 + 1), :]
            if k1 > 0:
                tr, ti = tw_ref[k1:k1 + 1, :], tw_ref[N1 + k1:N1 + k1 + 1, :]
                br, bi = br * tr + bi * ti, bi * tr - br * ti
            bs.append((br, bi))
        zs = _fft(bs, +1)
        for n in range(N1):
            c_scr[pl.ds(2 * LP * n + r0 + ro, SR), :] = zs[n][0]
            c_scr[pl.ds(2 * LP * n + LP + r0 + ro, SR), :] = zs[n][1]

    def head_body(t, carry):
        nc = S // KC
        seq = [(u, c) for u in range(HP) for c in range(nc)]
        qms = {}
        accs = {}
        r0 = pl.multiple_of(t * RG, 8)
        rp = pl.multiple_of(((t + H // HP - 1) % (H // HP)) * RG, 8)
        per = len(seq) // NSG
        for i in range(len(seq) + SKEW):
            j, ph = divmod(i, per)
            if j < NSG and ph == ST_X:
                if j == 0:
                    inv_stage(rp, NSG - 1)
                else:
                    inv_stage(r0, j - 1)
                fwd_stage(r0, j)
            if i < len(seq):
                u, c = seq[i]
                h = HP * t + u
                if c == 0:
                    qms[u] = masked_q(h, 0, S, True)
                qm, g0 = qms[u]
                s = _nn(k_scr[pl.ds(c * KC, KC), pl.ds(g0, 128)], qm)
                p_scr[i % (SKEW + 1)] = jnp.exp2(s).astype(BF16)
            if i >= SKEW:
                u, c = seq[i - SKEW]
                h = HP * t + u
                h0 = pl.multiple_of(h * 32, 32)
                ov = _nn(vt_scr[pl.ds(h0, 32), pl.ds(c * KC, KC)], p_scr[(i - SKEW) % (SKEW + 1)])
                accs[u] = ov if u not in accs else accs[u] + ov
                if c == nc - 1:
                    acc = accs[u]
                    l = acc[28:29, :]
                    l_scr[pl.ds(h, 1), :] = l
                    ot_scr[pl.ds(h0, 32), :] = (acc * (g_scr[...] / l)).astype(BF16)
            if j < NSG and ph == ST_X:
                x_stage()
            if j < NSG and ph == ST_Y:
                y_stage(r0, j)
        return carry

    fb_scr[...] = jnp.zeros(fb_scr.shape, F32)
    jax.lax.fori_loop(0, H // HP, head_body, 0)

    lv = l_scr[...]
    bad = jnp.where((lv >= L_LO) & (lv <= L_HI), 0.0, 1.0)
    nbad = jnp.max(bad)

    @pl.when(nbad > 0.5)
    def _():
        TQ = 128
        def item(it, carry):
            h = it // (S // TQ)
            q0 = pl.multiple_of((it % (S // TQ)) * TQ, TQ)
            h0 = pl.multiple_of(h * 32, 32)
            qm, g0 = masked_q(h, q0, TQ, False)
            s = _nn(k_scr[:, pl.ds(g0, 128)], qm)
            m = jnp.max(s, axis=0, keepdims=True)
            p = jnp.exp2(s - m).astype(BF16)
            acc = _nn(vt_scr[pl.ds(h0, 32), :], p)
            l = acc[28:29, :]
            ot_scr[pl.ds(h0, 32), pl.ds(q0, TQ)] = (acc * (g_scr[:, pl.ds(q0, TQ)] / l)).astype(BF16)
            return carry
        jax.lax.fori_loop(0, H * (S // TQ), item, 0)

    def zrows(a, b, c):
        nt = OW // 128
        return jnp.concatenate([c_scr[2 * LP * n + a:2 * LP * n + b, :] for n in range(c * nt, (c + 1) * nt)], axis=1)

    z4 = jnp.zeros((4, D), F32)

    def dinv(c):
        zc0 = jnp.concatenate([zrows(0, 64, c), zrows(LP, LP + 64, c)], axis=0).astype(BF16)
        zc2 = jnp.concatenate([zrows(64, 120, c), zrows(LP + 64, LP + 120, c)], axis=0).astype(BF16)
        zr13 = zrows(120, 232, c).astype(BF16)
        zi13 = zrows(LP + 120, LP + 232, c).astype(BF16)
        p0 = _nn(g02_v[0:112, :], zc0)
        p2 = _nn(g02_v[112:224, 0:112], zc2)
        pc = _nn(g13_v[0:112, :], zr13)
        qs = _nn(g13_v[112:240, :], zi13)
        aa = pc - qs[0:112]
        bb = _reflect(jnp.concatenate([-(pc + qs[0:112]), qs[112:120]], axis=0))
        pp, pm = p0 + p2, p0 - p2
        return jnp.concatenate([pp + aa, pm + bb, pp - aa, pm - bb], axis=0)

    wo = wo_v[...].astype(F32)
    parts = []
    for h in range(H):
        parts += [wo[DH * h: DH * h + DH, :], z4]
    wo_pad = jnp.concatenate(parts, axis=0)
    woT = jnp.concatenate([wo_pad, jnp.zeros((512, 64), F32)], axis=1).T[:D, :].astype(BF16)
    bts = {c: dinv(c) for c in range(DLEAD)}
    for c in range(OCH):
        cols = slice(c * OW, (c + 1) * OW)
        if c + DLEAD < OCH:
            bts[c + DLEAD] = dinv(c + DLEAD)
        at = _nn(woT, ot_scr[:, cols])
        res = at + (1.0 - g_scr[:, cols]) * bts.pop(c)
        out_v[:, cols] = res.astype(BF16)
        c_out[c].start()
    for c in c_out:
        c.wait()


@jax.jit
def pallas_gated_mix__softmax_full_mha__spectral_gfnet__prompt_kernel(A_x, A_wqkv, A_wo, B_x, B_w_r, B_w_i, gate_w):
    F02, F13, G02, G13, Mf, TW = _constants()
    hbm = pl.BlockSpec(memory_space=pltpu.MemorySpace.HBM)
    vmem = pl.BlockSpec(memory_space=pltpu.MemorySpace.VMEM)
    out = pl.pallas_call(
        _kernel,
        out_shape=jax.ShapeDtypeStruct((D, S), BF16),
        in_specs=[hbm, hbm, hbm, hbm, hbm, vmem, hbm, hbm, hbm, hbm, hbm, vmem],
        out_specs=hbm,
        scratch_shapes=[
            pltpu.VMEM((D, S), BF16),
            pltpu.VMEM((D, 512), BF16),
            pltpu.VMEM((D, 640), BF16),
            pltpu.VMEM((D, D), BF16),
            pltpu.VMEM((D, D), BF16),
            pltpu.VMEM((DF, S), BF16),
            pltpu.VMEM((DF, S), BF16),
            pltpu.VMEM(F02.shape, BF16),
            pltpu.VMEM(F13.shape, BF16),
            pltpu.VMEM(G02.shape, BF16),
            pltpu.VMEM(G13.shape, BF16),
            pltpu.VMEM(Mf.shape, BF16),
            pltpu.VMEM((D, S), BF16),
            pltpu.SemaphoreType.DMA((4 + XCH + 7 + OCH,)),
            pltpu.VMEM((S, 512), BF16),
            pltpu.VMEM((D + 16, S), BF16),
            pltpu.VMEM((512, S), BF16),
            pltpu.VMEM((H, S), F32),
            pltpu.VMEM((1, S), F32),
            pltpu.VMEM((H, S), F32),
            pltpu.VMEM((512, S), BF16),
            pltpu.VMEM((2 * LP, S), F32),
            pltpu.VMEM((N1 * 2 * LP + N1 * 2 * RG, 128), F32),
            pltpu.VMEM((2, S, 128), I32),
            pltpu.VMEM((N1, 256, 128), I32),
            pltpu.VMEM((N1, LP, 128), I32),
            pltpu.VMEM((N1 * 2 * RG, 128), BF16),
            pltpu.VMEM((N1 * 2 * RG, 128), F32),
            pltpu.VMEM((SKEW + 1, KC, S), BF16),
        ],
        compiler_params=pltpu.CompilerParams(vmem_limit_bytes=110 * 1024 * 1024),
    )(A_x.reshape(S, D).T, A_wqkv, A_wo, B_w_r.T, B_w_i.T, gate_w, F02, F13, G02, G13, Mf, TW)
    return out.T.reshape(1, S, D)
```

```python
import math
import numpy as np
import jax
import jax.numpy as jnp
from jax.experimental import pallas as pl
from jax.experimental.pallas import tpu as pltpu

S, D, H, DH = 2048, 448, 16, 28
DF = D // 2 + 1
LP = 256
N1, N2 = 16, 128
QSCALE = DH ** -0.5 * math.log2(math.e)
F32, BF16, I32 = jnp.float32, jnp.bfloat16, jnp.int32
L_LO, L_HI = 2.0 ** -64, 2.0 ** 64
CLS = ((0, 0, 64, 57), (2, 64, 56, 56), (1, 120, 56, 56), (3, 176, 56, 56))
NREAL = 232


def _constants():
    d0 = np.arange(112)[None, :]

    def cs(cls, n_real, n_pad):
        l = (cls + 4 * np.arange(n_real))[:, None]
        th = 2 * np.pi * ((l * d0) % D) / D
        c = np.zeros((n_pad, 112)); s = np.zeros((n_pad, 112))
        c[:n_real] = np.cos(th); s[:n_real] = np.sin(th)
        w = np.zeros((n_pad, 1)); w[:n_real] = 2.0
        w[:n_real][(l == 0) | (l == D // 2)] = 1.0
        return c, s, w
    c0, s0, w0 = cs(0, 57, 64); c2, s2, w2 = cs(2, 56, 56); c1, s1, w1 = cs(1, 56, 56); c3, s3, w3 = cs(3, 56, 56)
    F02 = np.concatenate([c0, -s0, c2, -s2], axis=0)
    F13 = np.zeros((224, 128))
    F13[0:56, :112] = c1; F13[56:112, :112] = c3
    F13[112:168, :112] = -s1; F13[168:224, :112] = -s3
    F13[112:168, 112] = -1.0; F13[168:224, 112] = 1.0
    nrm = 1.0 / (D * S)
    G0 = np.concatenate([(w0 * c0).T, (-w0 * s0).T], axis=1) * nrm
    G2 = np.concatenate([(w2 * c2).T, (-w2 * s2).T], axis=1) * nrm
    G13 = np.zeros((240, 112))
    G13[0:112] = np.concatenate([(w1 * c1).T, (w3 * c3).T], axis=1) * nrm
    G13[112:224] = np.concatenate([(w1 * s1).T, (w3 * s3).T], axis=1) * nrm
    G13[224] = np.concatenate([-w1[:, 0], w3[:, 0]]) * nrm
    G02 = np.zeros((224, 128)); G02[:112] = G0; G02[112:, :112] = G2
    n2 = np.arange(N2)[:, None]; k2 = np.arange(N2)[None, :]
    th = 2 * np.pi * ((n2 * k2) % N2) / N2
    FF = np.where(n2 <= N2 // 2, np.cos(th), np.sin(th))
    FF[0] *= 0.5; FF[N2 // 2] *= 0.5
    k1 = np.arange(N1)[:, None]
    tt = 2 * np.pi * ((k1 * np.arange(N2)[None, :]) % S) / S
    TW = np.concatenate([np.cos(tt), -np.sin(tt)], axis=0)
    return tuple(jnp.asarray(m, BF16) for m in (F02, F13, G02, G13, FF)) + (jnp.asarray(TW, F32),)


def _cmul_const(re, im, k, n, sign):
    k = k % n
    if k == 0:
        return re, im
    if 4 * k == n:
        return (-im, re) if sign > 0 else (im, -re)
    if 2 * k == n:
        return -re, -im
    if 4 * k == 3 * n:
        return (im, -re) if sign > 0 else (-im, re)
    c = math.cos(2 * math.pi * k / n); s = sign * math.sin(2 * math.pi * k / n)
    if (8 * k) % n == 0:
        a = abs(c)
        sc, ss = (1 if c > 0 else -1), (1 if s > 0 else -1)
        rr = (re - im) if sc == ss else (re + im)
        ii = (re + im) if sc == ss else (im - re)
        return rr * (sc * a), ii * (sc * a)
    return re * c - im * s, re * s + im * c


def _fft(xs, sign):
    n = len(xs)
    if n == 1:
        return xs
    ev = _fft(xs[0::2], sign)
    od = _fft(xs[1::2], sign)
    out = [None] * n
    for k in range(n // 2):
        tr, ti = _cmul_const(od[k][0], od[k][1], k, n, sign)
        out[k] = (ev[k][0] + tr, ev[k][1] + ti)
        out[k + n // 2] = (ev[k][0] - tr, ev[k][1] - ti)
    return out


def _nn(a, b):
    return jnp.dot(a, b, preferred_element_type=F32)


def _rev(x):
    lane = jax.lax.broadcasted_iota(I32, x.shape, 1)
    return jnp.take_along_axis(x, (N2 - lane) % N2, axis=1)


def _reflect(y):
    sub = jax.lax.broadcasted_iota(I32, (8, y.shape[1]), 0)
    idx = (8 - sub) % 8
    g = [jnp.take_along_axis(y[8 * j:8 * j + 8], idx, axis=0) for j in range(15)]
    return jnp.concatenate([jnp.where(sub == 0, g[14 - j], g[13 - j]) for j in range(14)], axis=0)


def _fold(re, im, sign):
    lane = jax.lax.broadcasted_iota(I32, re.shape, 1)
    lo = lane <= N2 // 2
    rr, ri = _rev(re), _rev(im)
    if sign < 0:
        return jnp.where(lo, re + rr, im - ri), jnp.where(lo, im + ri, rr - re)
    return jnp.where(lo, re + rr, ri - im), jnp.where(lo, im + ri, re - rr)


KC = 256
SKEW = 1
HP = 2
RG = LP // (H // HP)
BPOS = 3
DLEAD = 4
NSG = 4
ST_X = 0
ST_Y = 3
XCH = 4
XW = S // XCH
OCH = 16
OW = S // OCH


def _kernel(xa_hbm, wqkv_hbm, wo_hbm, wr_hbm, wi_hbm, gw_ref, f02_hbm, f13_hbm, g02_hbm, g13_hbm, mf_hbm, tw_ref,
            out_hbm,
            x_v, wq_v, wk_v, wv_v, wo_v, wr_v, wi_v, f02_v, f13_v, g02_v, g13_v, mf_v, out_v, sems,
            k_scr, qt_scr, vt_scr, negm_scr, g_scr, l_scr, ot_scr,
            u_scr, c_scr, wn_scr, wp_scr, wc_scr, fa_scr, fb_scr, p_scr):
    nsem = [0]

    def cp(src, dst):
        nsem[0] += 1
        return pltpu.make_async_copy(src, dst, sems.at[nsem[0] - 1])

    c_wq = cp(wqkv_hbm.at[:, pl.ds(0, 512)], wq_v)
    c_wk = cp(wqkv_hbm.at[:, pl.ds(384, 640)], wk_v)
    c_f = [cp(f02_hbm, f02_v), cp(f13_hbm, f13_v)]
    c_x = [cp(xa_hbm.at[:, pl.ds(c * XW, XW)], x_v.at[:, pl.ds(c * XW, XW)]) for c in range(XCH)]
    rest = [cp(wqkv_hbm.at[:, pl.ds(896, 448)], wv_v), cp(wr_hbm, wr_v), cp(wi_hbm, wi_v), cp(mf_hbm, mf_v),
            cp(wo_hbm, wo_v), cp(g02_hbm, g02_v), cp(g13_hbm, g13_v)]
    c_out = [cp(out_v.at[:, pl.ds(c * OW, OW)], out_hbm.at[:, pl.ds(c * OW, OW)]) for c in range(OCH)]
    c_wq.start()
    c_x[0].start()
    c_wq.wait()
    c_wk.start()
    for c in c_f:
        c.start()
    for c in c_x[1:]:
        c.start()

    wqT = jnp.concatenate([wq_v[...].astype(F32).T[0:D, :], gw_ref[...].astype(F32).reshape(1, D),
                           jnp.zeros((15, D), F32)], axis=0).astype(BF16)
    w_box = {}

    kmax = [None] * 4

    def dfwd_prep(c):
        cols = slice(c * XW, (c + 1) * XW)
        xf = x_v[:, cols].astype(F32)
        x0, x1, x2, x3 = (xf[112 * j:112 * j + 112] for j in range(4))
        s02, s13 = x0 + x2, x1 + x3
        e0 = (s02 + s13).astype(BF16)
        e2 = (s02 - s13).astype(BF16)
        a, b = x0 - x2, x1 - x3
        bt = _reflect(jnp.concatenate([b, jnp.zeros((8, XW), F32)], axis=0))
        pp = (a - bt).astype(BF16)
        mm = jnp.concatenate([a + bt, b[0:1], jnp.zeros((15, XW), F32)], axis=0).astype(BF16)
        return e0, e2, pp, mm

    def dfwd_mm(c, ops):
        cols = slice(c * XW, (c + 1) * XW)
        e0, e2, pp, mm = ops
        r0 = _nn(f02_v[0:128, :], e0)
        r2 = _nn(f02_v[128:240, :], e2)
        rc = _nn(f13_v[0:112, 0:112], pp)
        rs = _nn(f13_v[112:224, :], mm)
        zpad = jnp.zeros((LP - NREAL, XW), F32)
        u_scr[0:LP, cols] = jnp.concatenate([r0[0:64], r2[0:56], rc, zpad], axis=0)
        u_scr[LP:2 * LP, cols] = jnp.concatenate([r0[64:128], r2[56:112], rs, zpad], axis=0)

    def dfwd(c):
        dfwd_mm(c, dfwd_prep(c))

    def qproj(c):
        cols = slice(c * XW, (c + 1) * XW)
        qf = _nn(wqT, x_v[:, cols])
        g_scr[:, cols] = jax.nn.sigmoid(qf[D:D + 1, :])
        qt_scr[:, cols] = (qf * QSCALE).astype(BF16)

    def kproj(c):
        cols = slice(c * XW, (c + 1) * XW)
        kt = _nn(w_box["k"], x_v[:, cols])
        ones_rows = jnp.concatenate([jnp.ones((1, XW), F32), jnp.zeros((15, XW), F32)], axis=0)
        for g in range(4):
            kg = jnp.concatenate([kt[112 * g:112 * g + 112, :], ones_rows], axis=0).T
            k_scr[cols, 128 * g:128 * g + 128] = kg.astype(BF16)
            km = jnp.max(jnp.abs(kg), axis=0, keepdims=True)
            kmax[g] = km if kmax[g] is None else jnp.maximum(kmax[g], km)

    def qkproj(c):
        qproj(c)
        kproj(c)

    def wshuf_first():
        wrb = pltpu.bitcast(wr_v[...].astype(F32), I32)
        wib = pltpu.bitcast(wi_v[...].astype(F32), I32)
        wpk = wrb | jax.lax.shift_right_logical(wib, 16)
        wpk = jnp.concatenate([wpk, jnp.zeros((256 - DF, S), I32)], axis=0)
        wn = wpk.T
        wn_scr[0] = wn[:, 0:128]
        wn_scr[1] = wn[:, 128:256]

    def wshuf_second(k1):
        for t in range(2):
            wp_scr[k1, 128 * t:128 * t + 128, :] = wn_scr[t, pl.ds(k1, N2, stride=N1), :].T
        wc_scr[k1] = jnp.concatenate([wp_scr[k1, pl.ds(c, n, stride=4), :] for c, _, n, _ in CLS]
                                     + [jnp.zeros((LP - NREAL, 128), I32)], axis=0)

    c_x[0].wait()
    qproj(0)
    c_wk.wait()
    for cf in c_f:
        cf.wait()
    for cr in rest:
        cr.start()
    w_box["k"] = wk_v[...].astype(F32).T[64:64 + D, :].astype(BF16)
    dfwd(0)
    kproj(0)
    for c in range(1, XCH):
        c_x[c].wait()
    for c in range(1, XCH - 1):
        qkproj(c)
        dfwd(c)

    for cr in rest:
        cr.wait()

    qkproj(XCH - 1)
    dfwd(XCH - 1)
    wvT = wv_v[...].astype(F32).T.astype(BF16)
    wshuf_first()

    def bound():
        hh = jax.lax.broadcasted_iota(I32, (8, 128), 0)
        ll = jax.lax.broadcasted_iota(I32, (8, 128), 1)
        for g in range(4):
            ind = jnp.where((ll >= hh * DH) & (ll < hh * DH + DH) & (hh < 4), kmax[g] * 1.02, 0.0).astype(BF16)
            qa = pltpu.bitcast(pltpu.bitcast(qt_scr[112 * g:112 * g + 128, :], I32) & jnp.int32(0x7FFF7FFF), BF16)
            mt = _nn(ind, qa)
            negm_scr[4 * g:4 * g + 4, :] = -mt[0:4]

    tail_rows = jnp.concatenate([jnp.ones((1, XW), F32), jnp.zeros((3, XW), F32)], axis=0)
    for c in range(XCH):
        cols = slice(c * XW, (c + 1) * XW)
        vt = _nn(wvT, x_v[:, cols])
        for h in range(H):
            vt_scr[32 * h:32 * h + 32, cols] = jnp.concatenate(
                [vt[DH * h:DH * h + DH, :], tail_rows], axis=0).astype(BF16)
        for k1 in range(4 * c, 4 * c + 4):
            wshuf_second(k1)
        if c == BPOS:
            bound()

    def masked_q(h, q0, tq, with_shift):
        g = h // 4
        r0 = pl.multiple_of(g * 112, 16)
        g0 = pl.multiple_of(g * 128, 128)
        w0 = (h % 4) * (DH // 2)
        qw = pltpu.bitcast(qt_scr[pl.ds(r0, 128), pl.ds(q0, tq)], I32)
        rows = jax.lax.broadcasted_iota(I32, (64, tq), 0)
        qm = jnp.where((rows >= w0) & (rows < w0 + DH // 2), qw, 0)
        if with_shift:
            sh = negm_scr[pl.ds(h, 1), pl.ds(q0, tq)].astype(BF16).astype(F32)
            shw = jax.lax.shift_right_logical(pltpu.bitcast(sh, I32), 16)
            qm = jnp.where(rows == 56, shw, qm)
        return pltpu.bitcast(qm, BF16), g0

    FX0 = N1 * 2 * LP
    SR = RG // NSG
    PR = N1 * 2 * SR

    def fwd_stage(r0, j):
        ro = j * SR
        xs = [(u_scr[pl.ds(r0 + ro, SR), 128 * n:128 * n + 128],
               u_scr[pl.ds(LP + r0 + ro, SR), 128 * n:128 * n + 128]) for n in range(N1)]
        ys = _fft(xs, -1)
        for k1 in range(N1):
            ar, ai = ys[k1]
            if k1 > 0:
                tr, ti = tw_ref[k1:k1 + 1, :], tw_ref[N1 + k1:N1 + k1 + 1, :]
                ar, ai = ar * tr - ai * ti, ar * ti + ai * tr
            f1, f2 = _fold(ar, ai, -1)
            fa_scr[2 * SR * k1:2 * SR * (k1 + 1), :] = jnp.concatenate([f1, f2], axis=0).astype(BF16)

    def x_stage():
        c_scr[FX0:FX0 + PR, :] = _nn(fa_scr[0:PR, :], mf_v[...])

    def y_stage(r0, j):
        ro = j * SR
        ys_ = []
        for k1 in range(N1):
            xr = c_scr[FX0 + 2 * SR * k1:FX0 + 2 * SR * k1 + SR, :]
            xi = c_scr[FX0 + 2 * SR * k1 + SR:FX0 + 2 * SR * (k1 + 1), :]
            w = wc_scr[k1, pl.ds(r0 + ro, SR), :]
            wr = pltpu.bitcast(w & jnp.int32(-65536), F32)
            wi = pltpu.bitcast(jax.lax.shift_left(w, 16), F32)
            ys_ += list(_fold(xr * wr - xi * wi, xr * wi + xi * wr, +1))
        fb_scr[0:PR, :] = _nn(jnp.concatenate(ys_, axis=0).astype(BF16), mf_v[...])

    def inv_stage(r0, j):
        ro = j * SR
        bs = []
        for k1 in range(N1):
            br = fb_scr[2 * SR * k1:2 * SR * k1 + SR, :]
            bi = fb_scr[2 * SR * k1 + SR:2 * SR * (k1 + 1), :]
            if k1 > 0:
                tr, ti = tw_ref[k1:k1 + 1, :], tw_ref[N1 + k1:N1 + k1 + 1, :]
                br, bi = br * tr + bi * ti, bi * tr - br * ti
            bs.append((br, bi))
        zs = _fft(bs, +1)
        for n in range(N1):
            c_scr[pl.ds(2 * LP * n + r0 + ro, SR), :] = zs[n][0]
            c_scr[pl.ds(2 * LP * n + LP + r0 + ro, SR), :] = zs[n][1]

    def head_body(t, carry):
        nc = S // KC
        seq = [(u, c) for u in range(HP) for c in range(nc)]
        qms = {}
        accs = {}
        r0 = pl.multiple_of(t * RG, 8)
        rp = pl.multiple_of(((t + H // HP - 1) % (H // HP)) * RG, 8)
        per = len(seq) // NSG
        for i in range(len(seq) + SKEW):
            j, ph = divmod(i, per)
            if j < NSG and ph == ST_X:
                if j == 0:
                    inv_stage(rp, NSG - 1)
                else:
                    inv_stage(r0, j - 1)
                fwd_stage(r0, j)
            if i < len(seq):
                u, c = seq[i]
                h = HP * t + u
                if c == 0:
                    qms[u] = masked_q(h, 0, S, True)
                qm, g0 = qms[u]
                s = _nn(k_scr[pl.ds(c * KC, KC), pl.ds(g0, 128)], qm)
                p_scr[i % (SKEW + 1)] = jnp.exp2(s).astype(BF16)
            if i >= SKEW:
                u, c = seq[i - SKEW]
                h = HP * t + u
                h0 = pl.multiple_of(h * 32, 32)
                ov = _nn(vt_scr[pl.ds(h0, 32), pl.ds(c * KC, KC)], p_scr[(i - SKEW) % (SKEW + 1)])
                accs[u] = ov if u not in accs else accs[u] + ov
                if c == nc - 1:
                    acc = accs[u]
                    l = acc[28:29, :]
                    l_scr[pl.ds(h, 1), :] = l
                    ot_scr[pl.ds(h0, 32), :] = (acc * (g_scr[...] / l)).astype(BF16)
            if j < NSG and ph == ST_X:
                x_stage()
            if j < NSG and ph == ST_Y:
                y_stage(r0, j)
        return carry

    fb_scr[...] = jnp.zeros(fb_scr.shape, F32)
    jax.lax.fori_loop(0, H // HP, head_body, 0)

    def zrows(a, b, c):
        nt = OW // 128
        return jnp.concatenate([c_scr[2 * LP * n + a:2 * LP * n + b, :] for n in range(c * nt, (c + 1) * nt)], axis=1)

    z4 = jnp.zeros((4, D), F32)

    def dinv(c):
        zc0 = jnp.concatenate([zrows(0, 64, c), zrows(LP, LP + 64, c)], axis=0).astype(BF16)
        zc2 = jnp.concatenate([zrows(64, 120, c), zrows(LP + 64, LP + 120, c)], axis=0).astype(BF16)
        zr13 = zrows(120, 232, c).astype(BF16)
        zi13 = zrows(LP + 120, LP + 232, c).astype(BF16)
        p0 = _nn(g02_v[0:112, :], zc0)
        p2 = _nn(g02_v[112:224, 0:112], zc2)
        pc = _nn(g13_v[0:112, :], zr13)
        qs = _nn(g13_v[112:240, :], zi13)
        aa = pc - qs[0:112]
        bb = _reflect(jnp.concatenate([-(pc + qs[0:112]), qs[112:120]], axis=0))
        pp, pm = p0 + p2, p0 - p2
        return jnp.concatenate([pp + aa, pm + bb, pp - aa, pm - bb], axis=0)

    def final():
        wo = wo_v[...].astype(F32)
        parts = []
        for h in range(H):
            parts += [wo[DH * h: DH * h + DH, :], z4]
        wo_pad = jnp.concatenate(parts, axis=0)
        woT = jnp.concatenate([wo_pad, jnp.zeros((512, 64), F32)], axis=1).T[:D, :].astype(BF16)
        bts = {c: dinv(c) for c in range(DLEAD)}
        for c in range(OCH):
            cols = slice(c * OW, (c + 1) * OW)
            if c + DLEAD < OCH:
                bts[c + DLEAD] = dinv(c + DLEAD)
            at = _nn(woT, ot_scr[:, cols])
            res = at + (1.0 - g_scr[:, cols]) * bts.pop(c)
            out_v[:, cols] = res.astype(BF16)
            c_out[c].start()
        for c in c_out:
            c.wait()

    lv = l_scr[...]
    bad = jnp.where((lv >= L_LO) & (lv <= L_HI), 0.0, 1.0)
    nbad = jnp.max(bad)
    final()

    @pl.when(nbad > 0.5)
    def _():
        TQ = 128
        def item(it, carry):
            h = it // (S // TQ)
            q0 = pl.multiple_of((it % (S // TQ)) * TQ, TQ)
            h0 = pl.multiple_of(h * 32, 32)
            qm, g0 = masked_q(h, q0, TQ, False)
            s = _nn(k_scr[:, pl.ds(g0, 128)], qm)
            m = jnp.max(s, axis=0, keepdims=True)
            p = jnp.exp2(s - m).astype(BF16)
            acc = _nn(vt_scr[pl.ds(h0, 32), :], p)
            l = acc[28:29, :]
            ot_scr[pl.ds(h0, 32), pl.ds(q0, TQ)] = (acc * (g_scr[:, pl.ds(q0, TQ)] / l)).astype(BF16)
            return carry
        jax.lax.fori_loop(0, H * (S // TQ), item, 0)
        final()


@jax.jit
def pallas_gated_mix__softmax_full_mha__spectral_gfnet__prompt_kernel(A_x, A_wqkv, A_wo, B_x, B_w_r, B_w_i, gate_w):
    F02, F13, G02, G13, Mf, TW = _constants()
    hbm = pl.BlockSpec(memory_space=pltpu.MemorySpace.HBM)
    vmem = pl.BlockSpec(memory_space=pltpu.MemorySpace.VMEM)
    out = pl.pallas_call(
        _kernel,
        out_shape=jax.ShapeDtypeStruct((D, S), BF16),
        in_specs=[hbm, hbm, hbm, hbm, hbm, vmem, hbm, hbm, hbm, hbm, hbm, vmem],
        out_specs=hbm,
        scratch_shapes=[
            pltpu.VMEM((D, S), BF16),
            pltpu.VMEM((D, 512), BF16),
            pltpu.VMEM((D, 640), BF16),
            pltpu.VMEM((D, D), BF16),
            pltpu.VMEM((D, D), BF16),
            pltpu.VMEM((DF, S), BF16),
            pltpu.VMEM((DF, S), BF16),
            pltpu.VMEM(F02.shape, BF16),
            pltpu.VMEM(F13.shape, BF16),
            pltpu.VMEM(G02.shape, BF16),
            pltpu.VMEM(G13.shape, BF16),
            pltpu.VMEM(Mf.shape, BF16),
            pltpu.VMEM((D, S), BF16),
            pltpu.SemaphoreType.DMA((4 + XCH + 7 + OCH,)),
            pltpu.VMEM((S, 512), BF16),
            pltpu.VMEM((D + 16, S), BF16),
            pltpu.VMEM((512, S), BF16),
            pltpu.VMEM((H, S), F32),
            pltpu.VMEM((1, S), F32),
            pltpu.VMEM((H, S), F32),
            pltpu.VMEM((512, S), BF16),
            pltpu.VMEM((2 * LP, S), F32),
            pltpu.VMEM((N1 * 2 * LP + N1 * 2 * RG, 128), F32),
            pltpu.VMEM((2, S, 128), I32),
            pltpu.VMEM((N1, 256, 128), I32),
            pltpu.VMEM((N1, LP, 128), I32),
            pltpu.VMEM((N1 * 2 * RG, 128), BF16),
            pltpu.VMEM((N1 * 2 * RG, 128), F32),
            pltpu.VMEM((SKEW + 1, KC, S), BF16),
        ],
        compiler_params=pltpu.CompilerParams(vmem_limit_bytes=110 * 1024 * 1024),
    )(A_x.reshape(S, D).T, A_wqkv, A_wo, B_w_r.T, B_w_i.T, gate_w, F02, F13, G02, G13, Mf, TW)
    return out.T.reshape(1, S, D)
```

```python
import math
import numpy as np
import jax
import jax.numpy as jnp
from jax.experimental import pallas as pl
from jax.experimental.pallas import tpu as pltpu

S, D, H, DH = 2048, 448, 16, 28
DF = D // 2 + 1
LP = 256
N1, N2 = 16, 128
QSCALE = DH ** -0.5 * math.log2(math.e)
F32, BF16, I32 = jnp.float32, jnp.bfloat16, jnp.int32
L_LO, L_HI = 2.0 ** -64, 2.0 ** 64
CLS = ((0, 0, 64, 57), (2, 64, 56, 56), (1, 120, 56, 56), (3, 176, 56, 56))
NREAL = 232


def _constants():
    d0 = np.arange(112)[None, :]

    def cs(cls, n_real, n_pad):
        l = (cls + 4 * np.arange(n_real))[:, None]
        th = 2 * np.pi * ((l * d0) % D) / D
        c = np.zeros((n_pad, 112)); s = np.zeros((n_pad, 112))
        c[:n_real] = np.cos(th); s[:n_real] = np.sin(th)
        w = np.zeros((n_pad, 1)); w[:n_real] = 2.0
        w[:n_real][(l == 0) | (l == D // 2)] = 1.0
        return c, s, w
    c0, s0, w0 = cs(0, 57, 64); c2, s2, w2 = cs(2, 56, 56); c1, s1, w1 = cs(1, 56, 56); c3, s3, w3 = cs(3, 56, 56)
    F02 = np.concatenate([c0, -s0, c2, -s2], axis=0)
    F13 = np.zeros((224, 128))
    F13[0:56, :112] = c1; F13[56:112, :112] = c3
    F13[112:168, :112] = -s1; F13[168:224, :112] = -s3
    F13[112:168, 112] = -1.0; F13[168:224, 112] = 1.0
    nrm = 1.0 / (D * S)
    G0 = np.concatenate([(w0 * c0).T, (-w0 * s0).T], axis=1) * nrm
    G2 = np.concatenate([(w2 * c2).T, (-w2 * s2).T], axis=1) * nrm
    G13 = np.zeros((240, 112))
    G13[0:112] = np.concatenate([(w1 * c1).T, (w3 * c3).T], axis=1) * nrm
    G13[112:224] = np.concatenate([(w1 * s1).T, (w3 * s3).T], axis=1) * nrm
    G13[224] = np.concatenate([-w1[:, 0], w3[:, 0]]) * nrm
    G02 = np.zeros((224, 128)); G02[:112] = G0; G02[112:, :112] = G2
    n2 = np.arange(N2)[:, None]; k2 = np.arange(N2)[None, :]
    th = 2 * np.pi * ((n2 * k2) % N2) / N2
    FF = np.where(n2 <= N2 // 2, np.cos(th), np.sin(th))
    FF[0] *= 0.5; FF[N2 // 2] *= 0.5
    k1 = np.arange(N1)[:, None]
    tt = 2 * np.pi * ((k1 * np.arange(N2)[None, :]) % S) / S
    TW = np.concatenate([np.cos(tt), -np.sin(tt)], axis=0)
    return tuple(jnp.asarray(m, BF16) for m in (F02, F13, G02, G13, FF)) + (jnp.asarray(TW, F32),)


def _cmul_const(re, im, k, n, sign):
    k = k % n
    if k == 0:
        return re, im
    if 4 * k == n:
        return (-im, re) if sign > 0 else (im, -re)
    if 2 * k == n:
        return -re, -im
    if 4 * k == 3 * n:
        return (im, -re) if sign > 0 else (-im, re)
    c = math.cos(2 * math.pi * k / n); s = sign * math.sin(2 * math.pi * k / n)
    if (8 * k) % n == 0:
        a = abs(c)
        sc, ss = (1 if c > 0 else -1), (1 if s > 0 else -1)
        rr = (re - im) if sc == ss else (re + im)
        ii = (re + im) if sc == ss else (im - re)
        return rr * (sc * a), ii * (sc * a)
    return re * c - im * s, re * s + im * c


def _fft(xs, sign):
    n = len(xs)
    if n == 1:
        return xs
    ev = _fft(xs[0::2], sign)
    od = _fft(xs[1::2], sign)
    out = [None] * n
    for k in range(n // 2):
        tr, ti = _cmul_const(od[k][0], od[k][1], k, n, sign)
        out[k] = (ev[k][0] + tr, ev[k][1] + ti)
        out[k + n // 2] = (ev[k][0] - tr, ev[k][1] - ti)
    return out


def _nn(a, b):
    return jnp.dot(a, b, preferred_element_type=F32)


def _rev(x):
    lane = jax.lax.broadcasted_iota(I32, x.shape, 1)
    return jnp.take_along_axis(x, (N2 - lane) % N2, axis=1)


def _reflect(y):
    sub = jax.lax.broadcasted_iota(I32, (8, y.shape[1]), 0)
    idx = (8 - sub) % 8
    g = [jnp.take_along_axis(y[8 * j:8 * j + 8], idx, axis=0) for j in range(15)]
    return jnp.concatenate([jnp.where(sub == 0, g[14 - j], g[13 - j]) for j in range(14)], axis=0)


def _fold(re, im, sign):
    lane = jax.lax.broadcasted_iota(I32, re.shape, 1)
    lo = lane <= N2 // 2
    rr, ri = _rev(re), _rev(im)
    if sign < 0:
        return jnp.where(lo, re + rr, im - ri), jnp.where(lo, im + ri, rr - re)
    return jnp.where(lo, re + rr, ri - im), jnp.where(lo, im + ri, re - rr)


KC = 256
SKEW = 1
NRING = 3
HP = 2
RG = LP // (H // HP)
BPOS = 3
DLEAD = 4
NSG = 4
ST_X = 0
ST_Y = 3
XCH = 4
XW = S // XCH
OCH = 16
OW = S // OCH


def _kernel(xa_hbm, wqkv_hbm, wo_hbm, wr_hbm, wi_hbm, gw_ref, f02_hbm, f13_hbm, g02_hbm, g13_hbm, mf_hbm, tw_ref,
            out_hbm,
            x_v, wq_v, wk_v, wv_v, wo_v, wr_v, wi_v, f02_v, f13_v, g02_v, g13_v, mf_v, out_v, sems,
            k_scr, qt_scr, vt_scr, negm_scr, g_scr, l_scr, ot_scr,
            u_scr, c_scr, wn_scr, wp_scr, wc_scr, fa_scr, fb_scr, p_scr):
    nsem = [0]

    def cp(src, dst):
        nsem[0] += 1
        return pltpu.make_async_copy(src, dst, sems.at[nsem[0] - 1])

    c_wq = cp(wqkv_hbm.at[:, pl.ds(0, 512)], wq_v)
    c_wk = cp(wqkv_hbm.at[:, pl.ds(384, 640)], wk_v)
    c_f = [cp(f02_hbm, f02_v), cp(f13_hbm, f13_v)]
    c_x = [cp(xa_hbm.at[:, pl.ds(c * XW, XW)], x_v.at[:, pl.ds(c * XW, XW)]) for c in range(XCH)]
    rest = [cp(wqkv_hbm.at[:, pl.ds(896, 448)], wv_v), cp(wr_hbm, wr_v), cp(wi_hbm, wi_v), cp(mf_hbm, mf_v),
            cp(wo_hbm, wo_v), cp(g02_hbm, g02_v), cp(g13_hbm, g13_v)]
    c_out = [cp(out_v.at[:, pl.ds(c * OW, OW)], out_hbm.at[:, pl.ds(c * OW, OW)]) for c in range(OCH)]
    c_wq.start()
    c_x[0].start()
    c_wq.wait()
    c_wk.start()
    for c in c_f:
        c.start()
    for c in c_x[1:]:
        c.start()

    wqT = jnp.concatenate([wq_v[...].astype(F32).T[0:D, :], gw_ref[...].astype(F32).reshape(1, D),
                           jnp.zeros((15, D), F32)], axis=0).astype(BF16)
    w_box = {}

    kmax = [None] * 4

    def dfwd_prep(c):
        cols = slice(c * XW, (c + 1) * XW)
        xf = x_v[:, cols].astype(F32)
        x0, x1, x2, x3 = (xf[112 * j:112 * j + 112] for j in range(4))
        s02, s13 = x0 + x2, x1 + x3
        e0 = (s02 + s13).astype(BF16)
        e2 = (s02 - s13).astype(BF16)
        a, b = x0 - x2, x1 - x3
        bt = _reflect(jnp.concatenate([b, jnp.zeros((8, XW), F32)], axis=0))
        pp = (a - bt).astype(BF16)
        mm = jnp.concatenate([a + bt, b[0:1], jnp.zeros((15, XW), F32)], axis=0).astype(BF16)
        return e0, e2, pp, mm

    def dfwd_mm(c, ops):
        cols = slice(c * XW, (c + 1) * XW)
        e0, e2, pp, mm = ops
        r0 = _nn(f02_v[0:128, :], e0)
        r2 = _nn(f02_v[128:240, :], e2)
        rc = _nn(f13_v[0:112, 0:112], pp)
        rs = _nn(f13_v[112:224, :], mm)
        zpad = jnp.zeros((LP - NREAL, XW), F32)
        u_scr[0:LP, cols] = jnp.concatenate([r0[0:64], r2[0:56], rc, zpad], axis=0)
        u_scr[LP:2 * LP, cols] = jnp.concatenate([r0[64:128], r2[56:112], rs, zpad], axis=0)

    def dfwd(c):
        dfwd_mm(c, dfwd_prep(c))

    def qproj(c):
        cols = slice(c * XW, (c + 1) * XW)
        qf = _nn(wqT, x_v[:, cols])
        g_scr[:, cols] = jax.nn.sigmoid(qf[D:D + 1, :])
        qt_scr[:, cols] = (qf * QSCALE).astype(BF16)

    def kproj(c):
        cols = slice(c * XW, (c + 1) * XW)
        kt = _nn(w_box["k"], x_v[:, cols])
        ones_rows = jnp.concatenate([jnp.ones((1, XW), F32), jnp.zeros((15, XW), F32)], axis=0)
        for g in range(4):
            kg = jnp.concatenate([kt[112 * g:112 * g + 112, :], ones_rows], axis=0).T
            k_scr[cols, 128 * g:128 * g + 128] = kg.astype(BF16)
            km = jnp.max(jnp.abs(kg), axis=0, keepdims=True)
            kmax[g] = km if kmax[g] is None else jnp.maximum(kmax[g], km)

    def qkproj(c):
        qproj(c)
        kproj(c)

    def wshuf_first():
        wrb = pltpu.bitcast(wr_v[...].astype(F32), I32)
        wib = pltpu.bitcast(wi_v[...].astype(F32), I32)
        wpk = wrb | jax.lax.shift_right_logical(wib, 16)
        wpk = jnp.concatenate([wpk, jnp.zeros((256 - DF, S), I32)], axis=0)
        wn = wpk.T
        wn_scr[0] = wn[:, 0:128]
        wn_scr[1] = wn[:, 128:256]

    def wshuf_second(k1):
        for t in range(2):
            wp_scr[k1, 128 * t:128 * t + 128, :] = wn_scr[t, pl.ds(k1, N2, stride=N1), :].T
        wc_scr[k1] = jnp.concatenate([wp_scr[k1, pl.ds(c, n, stride=4), :] for c, _, n, _ in CLS]
                                     + [jnp.zeros((LP - NREAL, 128), I32)], axis=0)

    c_x[0].wait()
    qproj(0)
    c_wk.wait()
    for cf in c_f:
        cf.wait()
    for cr in rest:
        cr.start()
    w_box["k"] = wk_v[...].astype(F32).T[64:64 + D, :].astype(BF16)
    dfwd(0)
    kproj(0)
    for c in range(1, XCH):
        c_x[c].wait()
    for c in range(1, XCH - 1):
        qkproj(c)
        dfwd(c)

    for cr in rest:
        cr.wait()

    qkproj(XCH - 1)
    dfwd(XCH - 1)
    wvT = wv_v[...].astype(F32).T.astype(BF16)
    wshuf_first()

    def bound():
        hh = jax.lax.broadcasted_iota(I32, (8, 128), 0)
        ll = jax.lax.broadcasted_iota(I32, (8, 128), 1)
        for g in range(4):
            ind = jnp.where((ll >= hh * DH) & (ll < hh * DH + DH) & (hh < 4), kmax[g] * 1.02, 0.0).astype(BF16)
            qa = pltpu.bitcast(pltpu.bitcast(qt_scr[112 * g:112 * g + 128, :], I32) & jnp.int32(0x7FFF7FFF), BF16)
            mt = _nn(ind, qa)
            negm_scr[4 * g:4 * g + 4, :] = -mt[0:4]

    tail_rows = jnp.concatenate([jnp.ones((1, XW), F32), jnp.zeros((3, XW), F32)], axis=0)
    for c in range(XCH):
        cols = slice(c * XW, (c + 1) * XW)
        vt = _nn(wvT, x_v[:, cols])
        for h in range(H):
            vt_scr[32 * h:32 * h + 32, cols] = jnp.concatenate(
                [vt[DH * h:DH * h + DH, :], tail_rows], axis=0).astype(BF16)
        for k1 in range(4 * c, 4 * c + 4):
            wshuf_second(k1)
        if c == BPOS:
            bound()

    def masked_q(h, q0, tq, with_shift):
        g = h // 4
        r0 = pl.multiple_of(g * 112, 16)
        g0 = pl.multiple_of(g * 128, 128)
        w0 = (h % 4) * (DH // 2)
        qw = pltpu.bitcast(qt_scr[pl.ds(r0, 128), pl.ds(q0, tq)], I32)
        rows = jax.lax.broadcasted_iota(I32, (64, tq), 0)
        qm = jnp.where((rows >= w0) & (rows < w0 + DH // 2), qw, 0)
        if with_shift:
            sh = negm_scr[pl.ds(h, 1), pl.ds(q0, tq)].astype(BF16).astype(F32)
            shw = jax.lax.shift_right_logical(pltpu.bitcast(sh, I32), 16)
            qm = jnp.where(rows == 56, shw, qm)
        return pltpu.bitcast(qm, BF16), g0

    FX0 = N1 * 2 * LP
    SR = RG // NSG
    PR = N1 * 2 * SR

    def fwd_stage(r0, j):
        ro = j * SR
        xs = [(u_scr[pl.ds(r0 + ro, SR), 128 * n:128 * n + 128],
               u_scr[pl.ds(LP + r0 + ro, SR), 128 * n:128 * n + 128]) for n in range(N1)]
        ys = _fft(xs, -1)
        for k1 in range(N1):
            ar, ai = ys[k1]
            if k1 > 0:
                tr, ti = tw_ref[k1:k1 + 1, :], tw_ref[N1 + k1:N1 + k1 + 1, :]
                ar, ai = ar * tr - ai * ti, ar * ti + ai * tr
            f1, f2 = _fold(ar, ai, -1)
            fa_scr[2 * SR * k1:2 * SR * (k1 + 1), :] = jnp.concatenate([f1, f2], axis=0).astype(BF16)

    def x_stage():
        c_scr[FX0:FX0 + PR, :] = _nn(fa_scr[0:PR, :], mf_v[...])

    def y_stage(r0, j):
        ro = j * SR
        ys_ = []
        for k1 in range(N1):
            xr = c_scr[FX0 + 2 * SR * k1:FX0 + 2 * SR * k1 + SR, :]
            xi = c_scr[FX0 + 2 * SR * k1 + SR:FX0 + 2 * SR * (k1 + 1), :]
            w = wc_scr[k1, pl.ds(r0 + ro, SR), :]
            wr = pltpu.bitcast(w & jnp.int32(-65536), F32)
            wi = pltpu.bitcast(jax.lax.shift_left(w, 16), F32)
            ys_ += list(_fold(xr * wr - xi * wi, xr * wi + xi * wr, +1))
        fb_scr[0:PR, :] = _nn(jnp.concatenate(ys_, axis=0).astype(BF16), mf_v[...])

    def inv_stage(r0, j):
        ro = j * SR
        bs = []
        for k1 in range(N1):
            br = fb_scr[2 * SR * k1:2 * SR * k1 + SR, :]
            bi = fb_scr[2 * SR * k1 + SR:2 * SR * (k1 + 1), :]
            if k1 > 0:
                tr, ti = tw_ref[k1:k1 + 1, :], tw_ref[N1 + k1:N1 + k1 + 1, :]
                br, bi = br * tr + bi * ti, bi * tr - br * ti
            bs.append((br, bi))
        zs = _fft(bs, +1)
        for n in range(N1):
            c_scr[pl.ds(2 * LP * n + r0 + ro, SR), :] = zs[n][0]
            c_scr[pl.ds(2 * LP * n + LP + r0 + ro, SR), :] = zs[n][1]

    def head_body(t, carry):
        nc = S // KC
        seq = [(u, c) for u in range(HP) for c in range(nc)]
        qms = {}
        accs = {}
        r0 = pl.multiple_of(t * RG, 8)
        rp = pl.multiple_of(((t + H // HP - 1) % (H // HP)) * RG, 8)
        per = len(seq) // NSG
        for i in range(len(seq) + SKEW):
            j, ph = divmod(i, per)
            if j < NSG and ph == ST_X:
                if j == 0:
                    inv_stage(rp, NSG - 1)
                else:
                    inv_stage(r0, j - 1)
                fwd_stage(r0, j)
            if i < len(seq):
                u, c = seq[i]
                h = HP * t + u
                if c == 0:
                    qms[u] = masked_q(h, 0, S, True)
                qm, g0 = qms[u]
                s = _nn(k_scr[pl.ds(c * KC, KC), pl.ds(g0, 128)], qm)
                p_scr[i % NRING] = jnp.exp2(s).astype(BF16)
            if i >= SKEW:
                u, c = seq[i - SKEW]
                h = HP * t + u
                h0 = pl.multiple_of(h * 32, 32)
                ov = _nn(vt_scr[pl.ds(h0, 32), pl.ds(c * KC, KC)], p_scr[(i - SKEW) % NRING])
                accs[u] = ov if u not in accs else accs[u] + ov
                if c == nc - 1:
                    acc = accs[u]
                    l = acc[28:29, :]
                    l_scr[pl.ds(h, 1), :] = l
                    ot_scr[pl.ds(h0, 32), :] = (acc * (g_scr[...] / l)).astype(BF16)
            if j < NSG and ph == ST_X:
                x_stage()
            if j < NSG and ph == ST_Y:
                y_stage(r0, j)
        return carry

    fb_scr[...] = jnp.zeros(fb_scr.shape, F32)
    jax.lax.fori_loop(0, H // HP, head_body, 0)

    def zrows(a, b, c):
        nt = OW // 128
        return jnp.concatenate([c_scr[2 * LP * n + a:2 * LP * n + b, :] for n in range(c * nt, (c + 1) * nt)], axis=1)

    z4 = jnp.zeros((4, D), F32)

    def dinv(c):
        zc0 = jnp.concatenate([zrows(0, 64, c), zrows(LP, LP + 64, c)], axis=0).astype(BF16)
        zc2 = jnp.concatenate([zrows(64, 120, c), zrows(LP + 64, LP + 120, c)], axis=0).astype(BF16)
        zr13 = zrows(120, 232, c).astype(BF16)
        zi13 = zrows(LP + 120, LP + 232, c).astype(BF16)
        p0 = _nn(g02_v[0:112, :], zc0)
        p2 = _nn(g02_v[112:224, 0:112], zc2)
        pc = _nn(g13_v[0:112, :], zr13)
        qs = _nn(g13_v[112:240, :], zi13)
        aa = pc - qs[0:112]
        bb = _reflect(jnp.concatenate([-(pc + qs[0:112]), qs[112:120]], axis=0))
        pp, pm = p0 + p2, p0 - p2
        return jnp.concatenate([pp + aa, pm + bb, pp - aa, pm - bb], axis=0)

    def final():
        wo = wo_v[...].astype(F32)
        parts = []
        for h in range(H):
            parts += [wo[DH * h: DH * h + DH, :], z4]
        wo_pad = jnp.concatenate(parts, axis=0)
        woT = jnp.concatenate([wo_pad, jnp.zeros((512, 64), F32)], axis=1).T[:D, :].astype(BF16)
        bts = {c: dinv(c) for c in range(DLEAD)}
        for c in range(OCH):
            cols = slice(c * OW, (c + 1) * OW)
            if c + DLEAD < OCH:
                bts[c + DLEAD] = dinv(c + DLEAD)
            at = _nn(woT, ot_scr[:, cols])
            res = at + (1.0 - g_scr[:, cols]) * bts.pop(c)
            out_v[:, cols] = res.astype(BF16)
            c_out[c].start()
        for c in c_out:
            c.wait()

    lv = l_scr[...]
    bad = jnp.where((lv >= L_LO) & (lv <= L_HI), 0.0, 1.0)
    nbad = jnp.max(bad)
    final()

    @pl.when(nbad > 0.5)
    def _():
        TQ = 128
        def item(it, carry):
            h = it // (S // TQ)
            q0 = pl.multiple_of((it % (S // TQ)) * TQ, TQ)
            h0 = pl.multiple_of(h * 32, 32)
            qm, g0 = masked_q(h, q0, TQ, False)
            s = _nn(k_scr[:, pl.ds(g0, 128)], qm)
            m = jnp.max(s, axis=0, keepdims=True)
            p = jnp.exp2(s - m).astype(BF16)
            acc = _nn(vt_scr[pl.ds(h0, 32), :], p)
            l = acc[28:29, :]
            ot_scr[pl.ds(h0, 32), pl.ds(q0, TQ)] = (acc * (g_scr[:, pl.ds(q0, TQ)] / l)).astype(BF16)
            return carry
        jax.lax.fori_loop(0, H * (S // TQ), item, 0)
        final()


@jax.jit
def pallas_gated_mix__softmax_full_mha__spectral_gfnet__prompt_kernel(A_x, A_wqkv, A_wo, B_x, B_w_r, B_w_i, gate_w):
    F02, F13, G02, G13, Mf, TW = _constants()
    hbm = pl.BlockSpec(memory_space=pltpu.MemorySpace.HBM)
    vmem = pl.BlockSpec(memory_space=pltpu.MemorySpace.VMEM)
    out = pl.pallas_call(
        _kernel,
        out_shape=jax.ShapeDtypeStruct((D, S), BF16),
        in_specs=[hbm, hbm, hbm, hbm, hbm, vmem, hbm, hbm, hbm, hbm, hbm, vmem],
        out_specs=hbm,
        scratch_shapes=[
            pltpu.VMEM((D, S), BF16),
            pltpu.VMEM((D, 512), BF16),
            pltpu.VMEM((D, 640), BF16),
            pltpu.VMEM((D, D), BF16),
            pltpu.VMEM((D, D), BF16),
            pltpu.VMEM((DF, S), BF16),
            pltpu.VMEM((DF, S), BF16),
            pltpu.VMEM(F02.shape, BF16),
            pltpu.VMEM(F13.shape, BF16),
            pltpu.VMEM(G02.shape, BF16),
            pltpu.VMEM(G13.shape, BF16),
            pltpu.VMEM(Mf.shape, BF16),
            pltpu.VMEM((D, S), BF16),
            pltpu.SemaphoreType.DMA((4 + XCH + 7 + OCH,)),
            pltpu.VMEM((S, 512), BF16),
            pltpu.VMEM((D + 16, S), BF16),
            pltpu.VMEM((512, S), BF16),
            pltpu.VMEM((H, S), F32),
            pltpu.VMEM((1, S), F32),
            pltpu.VMEM((H, S), F32),
            pltpu.VMEM((512, S), BF16),
            pltpu.VMEM((2 * LP, S), F32),
            pltpu.VMEM((N1 * 2 * LP + N1 * 2 * RG, 128), F32),
            pltpu.VMEM((2, S, 128), I32),
            pltpu.VMEM((N1, 256, 128), I32),
            pltpu.VMEM((N1, LP, 128), I32),
            pltpu.VMEM((N1 * 2 * RG, 128), BF16),
            pltpu.VMEM((N1 * 2 * RG, 128), F32),
            pltpu.VMEM((NRING, KC, S), BF16),
        ],
        compiler_params=pltpu.CompilerParams(vmem_limit_bytes=110 * 1024 * 1024),
    )(A_x.reshape(S, D).T, A_wqkv, A_wo, B_w_r.T, B_w_i.T, gate_w, F02, F13, G02, G13, Mf, TW)
    return out.T.reshape(1, S, D)
```
